```python
import jax
import jax.numpy as jnp

def _softmax(x, axis=-1):
    return jax.nn.softmax(x, axis=axis)

def _gelu(x):
    return jax.nn.gelu(x, approximate=True)

def _silu(x):
    return jax.nn.silu(x)

def _sigmoid(x):
    return jax.nn.sigmoid(x)

def _layernorm(x, axis=-1, eps=1e-05):
    m = jnp.mean(x, axis=axis, keepdims=True)
    v = jnp.var(x, axis=axis, keepdims=True)
    return (x - m) / jnp.sqrt(v + eps)

def _scatter_add(tgt, idx, src, axis=0):
    return tgt.at[idx].add(src)

def _segment_sum(src, seg, n):
    return jax.ops.segment_sum(src, seg, n)

class _Rng:

    def __init__(self, key):
        self._k = key

    def _next(self):
        self._k, sub = jax.random.split(self._k)
        return sub

    def normal(self, shape):
        return jax.random.normal(self._next(), shape, dtype=jnp.bfloat16)

    def randint(self, lo, hi, shape):
        return jax.random.randint(self._next(), shape, lo, hi, dtype=jnp.int32)

    def uniform(self, shape, lo=0.0, hi=1.0):
        return jax.random.uniform(self._next(), shape, jnp.bfloat16, lo, hi)

    def permutation(self, n):
        return jax.random.permutation(self._next(), n)
kernel_name = 'adaLN_cond__compressed_kv_cla__mixer_s_mlp__prompt'

def setup_inputs():
    _rng = _Rng(jax.random.key(int.from_bytes(__import__("os").urandom(4), "little")))
    _w = lambda a: (lambda t: t.astype(jnp.bfloat16) if jnp.issubdtype(t.dtype, jnp.floating) else t)(jnp.asarray(a))

    def _A_setup():
        B, H, Sq, Sk, D, M = (1, 32, 2048, 2048, 128, 640)
        Dc = 4 * D
        return {'x': _w((lambda *s: _rng.normal(s) * 0.05)(B, Sq, M)), 'c_kv': _w((lambda *s: _rng.normal(s) * 0.05)(B, Sk, Dc)), 'w_q': _w((lambda *s: _rng.normal(s) * 0.05)(M, H, D) * M ** (-0.5)), 'w_uk': _w((lambda *s: _rng.normal(s) * 0.05)(Dc, H, D) * Dc ** (-0.5)), 'w_uv': _w((lambda *s: _rng.normal(s) * 0.05)(Dc, H, D) * Dc ** (-0.5)), 'w_o': _w((lambda *s: _rng.normal(s) * 0.05)(H, D, M) * (H * D) ** (-0.5))}
    _A_in = _A_setup()

    def _B_setup():
        B, S, D, F = (1, 2048, 640, 1728)
        return {'x': _w((lambda *s: _rng.normal(s) * 0.05)(B, S, D)), 'w1': _w((lambda *s: _rng.normal(s) * 0.05)(D, D) * D ** (-0.5)), 'w2': _w((lambda *s: _rng.normal(s) * 0.05)(D, D) * D ** (-0.5)), 'w3': _w((lambda *s: _rng.normal(s) * 0.05)(D, F) * D ** (-0.5)), 'w4': _w((lambda *s: _rng.normal(s) * 0.05)(F, D) * F ** (-0.5))}
    _B_in = _B_setup()
    return {'A_x': _A_in['x'], 'A_c_kv': _A_in['c_kv'], 'A_w_q': _A_in['w_q'], 'A_w_uk': _A_in['w_uk'], 'A_w_uv': _A_in['w_uv'], 'A_w_o': _A_in['w_o'], 'B_x': _B_in['x'], 'B_w1': _B_in['w1'], 'B_w2': _B_in['w2'], 'B_w3': _B_in['w3'], 'B_w4': _B_in['w4'], 'c': _w((lambda *s: _rng.normal(s) * 0.05)(1, 640)), 'w_mod': _w((lambda *s: _rng.normal(s) * 0.05)(640, 6 * 640) * 640 ** (-0.5))}

def reference(A_x, A_c_kv, A_w_q, A_w_uk, A_w_uv, A_w_o, B_x, B_w1, B_w2, B_w3, B_w4, c, w_mod):

    def _A_ref(x, c_kv, w_q, w_uk, w_uv, w_o):
        B, Sq, M = (x.shape[0], x.shape[1], x.shape[2])
        Sk = c_kv.shape[1]
        H, D = (w_q.shape[1], w_q.shape[2])
        q = jnp.einsum('bqm,mhd->bhqd', x, w_q)
        k = jnp.einsum('bkc,chd->bhkd', c_kv, w_uk)
        v = jnp.einsum('bkc,chd->bhkd', c_kv, w_uv)
        scores = jnp.einsum('bhqd,bhkd->bhqk', q, k) * D ** (-0.5)
        off = Sk - Sq
        qi = jnp.arange(Sq)[:, None]
        kj = jnp.arange(Sk)[None, :]
        cmask = kj <= qi + off
        scores = jnp.where(cmask[None, None], scores, -1000000000.0)
        p = _softmax(scores, axis=-1)
        ctx = jnp.einsum('bhqk,bhkd->bhqd', p, v)
        return jnp.einsum('bhqd,hdm->bqm', ctx, w_o)

    def _B_ref(x, w1, w2, w3, w4):
        B, S, D = x.shape
        h = _gelu(_layernorm(x, axis=-1) @ w1)
        c = D // 4
        g0 = jnp.pad(h[:, :, 0 * c:1 * c], ((0, 0), (1, 0), (0, 0)))[:, :S, :]
        g1 = jnp.pad(h[:, :, 1 * c:2 * c], ((0, 0), (0, 1), (0, 0)))[:, 1:, :]
        g2 = jnp.pad(h[:, :, 2 * c:3 * c], ((0, 0), (2, 0), (0, 0)))[:, :S, :]
        g3 = jnp.pad(h[:, :, 3 * c:], ((0, 0), (0, 2), (0, 0)))[:, 2:, :]
        hs = jnp.concatenate([g0, g1, g2, g3], axis=-1) @ w2
        x1 = x + hs
        h2 = _gelu(_layernorm(x1, axis=-1) @ w3) @ w4
        return x1 + h2
    x = A_x
    mod = (_silu(c) @ w_mod).reshape(c.shape[0], 6, 1, -1)
    sa, ca, ga, sb, cb, gb = (mod[:, 0].copy(), mod[:, 1].copy(), mod[:, 2].copy(), mod[:, 3].copy(), mod[:, 4].copy(), mod[:, 5].copy())
    h = _layernorm(x, axis=-1) * (1 + ca) + sa
    x = x + ga * _A_ref(h, A_c_kv, A_w_q, A_w_uk, A_w_uv, A_w_o)
    h = _layernorm(x, axis=-1) * (1 + cb) + sb
    x = x + gb * _B_ref(h, B_w1, B_w2, B_w3, B_w4)
    return x
```

```python
import functools
import math

import jax
import jax.numpy as jnp
import jax.experimental.pallas as pl
import jax.experimental.pallas.tpu as pltpu

S = 2048
M = 640
H = 32
D = 128
DC = 4 * D
F = 1728
HG = 8
NG = H // HG
HC = 1
NP = H // HC
PPG = HG // HC
BQ = 256
NB = S // BQ
KC = 256
TPOS = 0
LAG = 4
BM = 256
FC = 512
PAD = 8
EPS = 1e-05
LOG2E = math.log2(math.e)
NT = (((1,), (1,)), ((), ()))
NEG = -1000000000.0 * LOG2E
QSCALE = (D ** -0.5) * LOG2E
bf16 = jnp.bfloat16
f32 = jnp.float32


def _mm(a, b):
    return jnp.dot(a, b, preferred_element_type=f32)


def _mm_nt(a, b):
    return jax.lax.dot_general(a, b, NT, preferred_element_type=f32)


def _ln(x):
    m = jnp.mean(x, axis=-1, keepdims=True)
    xc = x - m
    v = jnp.mean(xc * xc, axis=-1, keepdims=True)
    return xc * jax.lax.rsqrt(v + EPS)


def _gelu(x):
    k0 = math.sqrt(2.0 / math.pi)
    return 0.5 * x * (1.0 + jnp.tanh(k0 * (x + 0.044715 * (x * x * x))))


def _kernel(c_ref, x_hbm, ckv_hbm, wq_hbm, wuk_hbm, wuv_hbm, wo_hbm,
            w1_hbm, w2_hbm, w3_hbm, w4_hbm, wmod_hbm,
            out_hbm,
            x_v, ckv_v, wq_raw0, wuk_raw0, wuv_raw0, wq_raw, wuk_raw, wuv_raw, wo_v,
            w1_v, w2_v, w3_v, w4_v, wmod_v,
            wq_t, wuk_t, wuv_t,
            mod_s, h_s, q_s, k_s, v_s, ctx_s, acc_s, hb_s, g_s, out_v, sems, wsems):
    def cp(i, src, dst):
        return pltpu.make_async_copy(src, dst, sems.at[i])

    cp_wmoda = cp(0, wmod_hbm.at[:, 0:2 * M], wmod_v.at[:, 0:2 * M])
    cp_x = cp(1, x_hbm, x_v)
    cp_ckv = cp(2, ckv_hbm, ckv_v)
    cp_wuk0 = cp(3, wuk_hbm.at[:, 0:HG, :], wuk_raw0)
    cp_wuv0 = cp(4, wuv_hbm.at[:, 0:HG, :], wuv_raw0)
    cp_wq0 = cp(5, wq_hbm.at[:, 0:HG, :], wq_raw0)
    cp_wmodb = cp(6, wmod_hbm.at[:, 2 * M:6 * M], wmod_v.at[:, 2 * M:6 * M])
    cp_w1 = cp(7, w1_hbm, w1_v)
    cp_w2 = cp(8, w2_hbm, w2_v)
    cp_w3 = cp(9, w3_hbm, w3_v)
    cp_w4 = cp(10, w4_hbm, w4_v)

    MQ, MK = M // PPG, DC // PPG

    def raw_copies(g):
        slot = g % 2
        h0 = pl.multiple_of((g // PPG + 1) * HG, HG)
        cidx = g % PPG
        return [
            pltpu.make_async_copy(wq_hbm.at[pl.ds(cidx * MQ, MQ), pl.ds(h0, HG), :],
                                  wq_raw.at[slot], wsems.at[slot, 0]),
            pltpu.make_async_copy(wuk_hbm.at[pl.ds(cidx * MK, MK), pl.ds(h0, HG), :],
                                  wuk_raw.at[slot], wsems.at[slot, 1]),
            pltpu.make_async_copy(wuv_hbm.at[pl.ds(cidx * MK, MK), pl.ds(h0, HG), :],
                                  wuv_raw.at[slot], wsems.at[slot, 2]),
        ]

    def wo_copy(g):
        return pltpu.make_async_copy(wo_hbm.at[g], wo_v.at[g], wsems.at[g % 2, 3])

    cp_wmoda.start()
    cp_x.start()
    acc_s[...] = jnp.zeros((S, M), f32)
    ctx_s[...] = jnp.zeros((S, HC * D), bf16)
    g_s[0:PAD, :] = jnp.zeros((PAD, M), f32)
    g_s[PAD + S:PAD + S + PAD, :] = jnp.zeros((PAD, M), f32)

    cv = jnp.broadcast_to(c_ref[...].astype(f32), (16, M))
    sil = (cv * jax.nn.sigmoid(cv)).astype(bf16)
    cp_wmoda.wait()
    cp_wq0.start()
    cp_wuk0.start()
    mod_s[:, 0:2 * M] = _mm(sil, wmod_v[:, 0:2 * M])[0:8, :]

    def mod(i):
        return mod_s[0:1, i * M:(i + 1) * M]

    cp_x.wait()
    cp_wuv0.start()
    cp_ckv.start()
    sa, ca = mod(0), mod(1)
    for r in range(NB):
        xr = x_v[r * BQ:(r + 1) * BQ, :].astype(f32)
        h_s[r * BQ:(r + 1) * BQ, :] = ((_ln(xr) * (1.0 + ca) + sa) * QSCALE).astype(bf16)

    for n, (cpw, raw, dst) in enumerate(((cp_wq0, wq_raw0, wq_t), (cp_wuk0, wuk_raw0, wuk_t),
                                         (cp_wuv0, wuv_raw0, wuv_t))):
        cpw.wait()
        if n == 2:
            wo_copy(0).start()
            for c_ in raw_copies(0):
                c_.start()
        t = jnp.swapaxes(raw[...], 0, 1)
        for j in range(HG):
            dst[j // HC, :, (j % HC) * D:(j % HC + 1) * D] = t[j]
    cp_ckv.wait()

    NRAW = NP - PPG

    def group(g, carry):
        wo_copy(g).wait()

        @pl.when(g < NRAW)
        def _():
            for c_ in raw_copies(g):
                c_.wait()

        @pl.when(g + 1 < NRAW)
        def _():
            for c_ in raw_copies(g + 1):
                c_.start()

        @pl.when(g + 1 < NP)
        def _():
            wo_copy(g + 1).start()

        for gi, c_ in enumerate((cp_wmodb, cp_w1, cp_w2, cp_w3, cp_w4)):
            pl.when(g == gi + 1)(c_.start)

        st = {}

        def pq(i):
            lo, hi = i * BQ, (i + 1) * BQ
            q_s[lo:hi, :] = _mm(h_s[lo:hi, :], wq_t[g]).astype(bf16)

        def pk(i):
            lo, hi = i * BQ, (i + 1) * BQ
            k_s[lo:hi, :] = _mm(ckv_v[lo:hi, :], wuk_t[g]).astype(bf16)

        def pv(i):
            lo, hi = i * BQ, (i + 1) * BQ
            v_s[lo:hi, :] = _mm(ckv_v[lo:hi, :], wuv_t[g]).astype(bf16)

        def po(i, gg):
            lo, hi = i * BQ, (i + 1) * BQ
            acc_s[lo:hi, :] += _mm(ctx_s[lo:hi, :], wo_v[gg])

        def nkc(i):
            return i * BQ // KC

        def qk_chunk(i, j, c):
            lo = i * BQ
            cl, ch = j * D, (j + 1) * D
            d = st.setdefault((i, j), dict(s=[], mx=None))
            if c == 0:
                d['q'] = q_s[lo:lo + BQ, cl:ch]
            q = d['q']
            if c < nkc(i):
                sc = _mm_nt(q, k_s[c * KC:(c + 1) * KC, cl:ch])
                d['s'].append(sc)
                t = functools.reduce(jnp.maximum, [sc[:, u:u + D] for u in range(0, KC, D)])
                d['mx'] = t if d['mx'] is None else jnp.maximum(d['mx'], t)
            else:
                r = jax.lax.broadcasted_iota(jnp.int32, (D, D), 0)
                cc = jax.lax.broadcasted_iota(jnp.int32, (D, D), 1)
                tri = cc <= r
                mx = d['mx']
                tiles = []
                for t in range(BQ // D):
                    st_ = _mm_nt(q[t * D:], k_s[lo + t * D:lo + (t + 1) * D, cl:ch])
                    top = jnp.where(tri, st_[:D], NEG)
                    st_ = top if t == BQ // D - 1 else jnp.concatenate([top, st_[D:]], axis=0)
                    tiles.append(st_)
                    if mx is None:
                        mx = st_
                    elif t == 0:
                        mx = jnp.maximum(mx, st_)
                    else:
                        mx = jnp.concatenate([mx[:t * D], jnp.maximum(mx[t * D:], st_)], axis=0)
                d['s'].append(tiles)
                d['m'] = jnp.max(mx, axis=1, keepdims=True)

        def epv_chunk(i, j, c):
            lo = i * BQ
            cl, ch = j * D, (j + 1) * D
            d = st[(i, j)]
            m = d['m']
            if c < nkc(i):
                sc = d['s'][c]
                ps = [jnp.exp2(sc[:, u:u + D] - m) for u in range(0, KC, D)]
                pb = jnp.concatenate([p_.astype(bf16) for p_ in ps], axis=1)
                o = _mm(pb, v_s[c * KC:(c + 1) * KC, cl:ch])
                d['acc'] = o if c == 0 else d['acc'] + o
                t = functools.reduce(jnp.add, ps)
                d['l'] = t if c == 0 else d['l'] + t
            else:
                l = d['l'] if c > 0 else None
                acc = d['acc'] if c > 0 else None
                for t, st_ in enumerate(d['s'][c]):
                    p = jnp.exp2(st_ - m[t * D:])
                    o = _mm(p.astype(bf16), v_s[lo + t * D:lo + (t + 1) * D, cl:ch])
                    if l is None:
                        l, acc = p, o
                    elif t == 0:
                        l, acc = l + p, acc + o
                    else:
                        l = jnp.concatenate([l[:t * D], l[t * D:] + p], axis=0)
                        acc = jnp.concatenate([acc[:t * D], acc[t * D:] + o], axis=0)
                lsum = jnp.sum(l, axis=1, keepdims=True)
                ctx_s[lo:lo + BQ, cl:ch] = (acc / lsum).astype(bf16)

        def phase(qk_unit, epv_unit, fillers):
            nq = nkc(qk_unit[0]) + 1 if qk_unit is not None else 0
            ne = nkc(epv_unit[0]) + 1 if epv_unit is not None else 0
            n = max(nq, ne)
            nf = len(fillers)
            fpos = [((2 * t + 1) * n) // (2 * nf) for t in range(nf)]
            for c in range(n):
                if c < nq:
                    qk_chunk(qk_unit[0], qk_unit[1], c)
                for t in range(nf):
                    if fpos[t] == c:
                        fillers[t]()
                if c < ne:
                    epv_chunk(epv_unit[0], epv_unit[1], c)

        def relayout():
            slot = g % 2
            cidx = g % PPG
            for raw, dst, mc in ((wq_raw, wq_t, MQ), (wuk_raw, wuk_t, MK), (wuv_raw, wuv_t, MK)):
                t = jnp.swapaxes(raw[slot], 0, 1)
                r0 = pl.multiple_of(cidx * mc, 16)
                for j in range(HG):
                    pidx = ((g // PPG + 1) * PPG + j) % NP
                    dst[pidx, pl.ds(r0, mc), :] = t[j]

        P = functools.partial
        pq(NB - 1)
        for c in range(LAG):
            pk(c)
        po(0, jnp.maximum(g - 1, 0))
        pq(NB - 2)
        R = BQ // KC
        for c in range(NB):
            if c + LAG < NB:
                pk(c + LAG)
            for cc_ in range(c * R, (c + 1) * R if c < NB - 1 else c * R + 1):
                qk_chunk(NB - 1, 0, cc_)
            pv(c)
        for i in reversed(range(NB)):
            f = []
            if i >= 2:
                f += [P(pq, i - 2)]
            if i + 1 < NB:
                f += [P(po, i + 1, g)]
            if i == TPOS:
                f += [relayout]
            phase((i - 1, 0) if i > 0 else None, (i, 0), f)
        return carry

    jax.lax.fori_loop(0, NP, group, 0)
    acc_s[0:BQ, :] += _mm(ctx_s[0:BQ, :], wo_v[NP - 1])

    cp_wmodb.wait()
    mod_s[:, 2 * M:6 * M] = _mm(sil, wmod_v[:, 2 * M:6 * M])[0:8, :]
    ga, sb, cb, gb = mod(2), mod(3), mod(4), mod(5)
    cp_w1.wait()
    cp_w2.wait()
    cp_w3.wait()
    cp_w4.wait()
    NR = S // BM
    lane = jax.lax.broadcasted_iota(jnp.int32, (BM, 128), 1)
    cp_out = [cp(11 + r, out_v.at[r * BM:(r + 1) * BM, :], out_hbm.at[0, r * BM:(r + 1) * BM, :])
              for r in range(NR)]
    fchunks = [(lo, min(lo + FC, F)) for lo in range(0, F, FC)]
    sv = {}

    def stage1(r):
        lo, hi = r * BM, (r + 1) * BM
        x1 = x_v[lo:hi, :].astype(f32) + ga * acc_s[lo:hi, :]
        hb = _ln(x1) * (1.0 + cb) + sb
        acc_s[lo:hi, :] = x1
        hb_s[lo:hi, :] = hb
        u = _ln(hb).astype(bf16)
        g_s[PAD + lo:PAD + hi, :] = _gelu(_mm(u, w1_v[...]))

    def mix(r):
        lo, hi = r * BM, (r + 1) * BM

        def sh(d, t):
            return g_s[PAD + lo + d:PAD + hi + d, t * 128:(t + 1) * 128]

        t0 = sh(-1, 0)
        t1 = jnp.where(lane < 32, sh(-1, 1), sh(1, 1))
        t2 = jnp.where(lane < 64, sh(1, 2), sh(-2, 2))
        t3 = jnp.where(lane < 96, sh(-2, 3), sh(2, 3))
        t4 = sh(2, 4)
        gs = jnp.concatenate([t0, t1, t2, t3, t4], axis=1).astype(bf16)
        sv[r] = dict(xb=hb_s[lo:hi, :] + _mm(gs, w2_v[...]))

    def norm(r):
        sv[r]['u'] = _ln(sv[r]['xb']).astype(bf16)

    def up(r, c):
        lo, hi = fchunks[c]
        sv[r][('h', c)] = _mm_nt(sv[r]['u'], w3_v[lo:hi, :])

    def down(r, c):
        lo, hi = fchunks[c]
        o = _mm(_gelu(sv[r][('h', c)]).astype(bf16), w4_v[lo:hi, :])
        sv[r]['o'] = o if c == 0 else sv[r]['o'] + o

    def finish(r):
        lo, hi = r * BM, (r + 1) * BM
        out_v[lo:hi, :] = (acc_s[lo:hi, :] + gb * (sv[r]['xb'] + sv[r]['o'])).astype(bf16)
        cp_out[r].start()

    nc = len(fchunks)
    for r in range(min(2, NR)):
        stage1(r)
    mix(0)
    norm(0)
    for r in range(NR):
        up(r, 0)
        for c in range(nc):
            if c + 1 < nc:
                up(r, c + 1)
            if c == 0 and r + 2 < NR:
                stage1(r + 2)
            if c == 1 and r + 1 < NR:
                mix(r + 1)
            if c == 2 and r + 1 < NR:
                norm(r + 1)
            down(r, c)
        finish(r)
    for r in range(NR):
        cp_out[r].wait()


@jax.jit
def pallas_adaLN_cond__compressed_kv_cla__mixer_s_mlp__prompt_kernel(
    A_x: jax.Array,
    A_c_kv: jax.Array,
    A_w_q: jax.Array,
    A_w_uk: jax.Array,
    A_w_uv: jax.Array,
    A_w_o: jax.Array,
    B_x: jax.Array,
    B_w1: jax.Array,
    B_w2: jax.Array,
    B_w3: jax.Array,
    B_w4: jax.Array,
    c: jax.Array,
    w_mod: jax.Array,
):
    del B_x
    any_spec = pl.BlockSpec(memory_space=pltpu.HBM)
    V = pltpu.VMEM
    scratch = [
        V((S, M), bf16), V((S, DC), bf16),
        V((M, HG, D), bf16), V((DC, HG, D), bf16), V((DC, HG, D), bf16),
        V((2, M // PPG, HG, D), bf16), V((2, DC // PPG, HG, D), bf16), V((2, DC // PPG, HG, D), bf16),
        V((NP, HC * D, M), bf16),
        V((M, M), bf16), V((M, M), bf16), V((F, M), bf16), V((F, M), bf16), V((M, 6 * M), bf16),
        V((NP, M, HC * D), bf16), V((NP, DC, HC * D), bf16), V((NP, DC, HC * D), bf16),
        V((8, 6 * M), f32), V((S, M), bf16),
        V((S, HC * D), bf16), V((S, HC * D), bf16), V((S, HC * D), bf16), V((S, HC * D), bf16),
        V((S, M), f32), V((S, M), f32), V((S + 2 * PAD, M), f32), V((S, M), bf16),
        pltpu.SemaphoreType.DMA((11 + S // BM,)),
        pltpu.SemaphoreType.DMA((2, 4)),
    ]
    out = pl.pallas_call(
        _kernel,
        out_shape=jax.ShapeDtypeStruct((1, S, M), bf16),
        in_specs=[pl.BlockSpec(memory_space=pltpu.VMEM)] + [any_spec] * 11,
        out_specs=any_spec,
        scratch_shapes=scratch,
        compiler_params=pltpu.CompilerParams(vmem_limit_bytes=120 * 1024 * 1024),
    )(c, A_x.reshape(S, M), A_c_kv.reshape(S, DC), A_w_q, A_w_uk, A_w_uv, A_w_o.reshape(NP, HC * D, M),
      B_w1, B_w2, B_w3.T, B_w4, w_mod)
    return out
```

```python
import functools
import math

import jax
import jax.numpy as jnp
import jax.experimental.pallas as pl
import jax.experimental.pallas.tpu as pltpu

S = 2048
M = 640
H = 32
D = 128
DC = 4 * D
F = 1728
HG = 8
NG = H // HG
HC = 1
NP = H // HC
PPG = HG // HC
BQ = 256
NB = S // BQ
KC = 256
ORDER = (7, 6, 5, 4, 3, 2, 0, 1)
TPOS = 7
LAG = 3
BM = 128
FC = 512
PAD = 8
EPS = 1e-05
LOG2E = math.log2(math.e)
NT = (((1,), (1,)), ((), ()))
NEG = -1000000000.0 * LOG2E
QSCALE = (D ** -0.5) * LOG2E
bf16 = jnp.bfloat16
f32 = jnp.float32


def _mm(a, b):
    return jnp.dot(a, b, preferred_element_type=f32)


def _mm_nt(a, b):
    return jax.lax.dot_general(a, b, NT, preferred_element_type=f32)


def _ln(x):
    m = jnp.mean(x, axis=-1, keepdims=True)
    xc = x - m
    v = jnp.mean(xc * xc, axis=-1, keepdims=True)
    return xc * jax.lax.rsqrt(v + EPS)


def _gelu(x):
    k0 = math.sqrt(2.0 / math.pi)
    return 0.5 * x * (1.0 + jnp.tanh(k0 * (x + 0.044715 * (x * x * x))))


def _kernel(c_ref, x_hbm, ckv_hbm, wq_hbm, wuk_hbm, wuv_hbm, wo_hbm,
            w1_hbm, w2_hbm, w3_hbm, w4_hbm, wmod_hbm,
            out_hbm,
            x_v, ckv_v, wq_raw0, wuk_raw0, wuv_raw0, wq_raw, wuk_raw, wuv_raw, wo_v,
            w1_v, w2_v, w3_v, w4_v, wmod_v,
            wq_t, wuk_t, wuv_t,
            mod_s, h_s, q_s, k_s, v_s, ctx_s, acc_s, hb_s, g_s, out_v, sems, wsems):
    def cp(i, src, dst):
        return pltpu.make_async_copy(src, dst, sems.at[i])

    XC = 4
    XR = S // XC
    cp_wmoda = [cp(t, wmod_hbm.at[t * (M // 2):(t + 1) * (M // 2), 0:2 * M],
                   wmod_v.at[t * (M // 2):(t + 1) * (M // 2), 0:2 * M]) for t in range(2)]
    cp_x = [cp(2 + t, x_hbm.at[t * XR:(t + 1) * XR, :], x_v.at[t * XR:(t + 1) * XR, :])
            for t in range(XC)]
    cp_ckv = [cp(6 + t, ckv_hbm.at[t * (S // 2):(t + 1) * (S // 2), :],
                 ckv_v.at[t * (S // 2):(t + 1) * (S // 2), :]) for t in range(2)]
    cp_wuk0 = cp(8, wuk_hbm.at[:, 0:HG, :], wuk_raw0)
    cp_wuv0 = cp(9, wuv_hbm.at[:, 0:HG, :], wuv_raw0)
    cp_wq0 = cp(10, wq_hbm.at[:, 0:HG, :], wq_raw0)
    cp_wmodb = cp(11, wmod_hbm.at[:, 2 * M:6 * M], wmod_v.at[:, 2 * M:6 * M])
    cp_w1 = cp(12, w1_hbm, w1_v)
    cp_w2 = cp(13, w2_hbm, w2_v)
    cp_w3 = cp(14, w3_hbm, w3_v)
    cp_w4 = cp(15, w4_hbm, w4_v)

    MQ, MK = M // PPG, DC // PPG

    def raw_copies(g):
        slot = g % 2
        h0 = pl.multiple_of((g // PPG + 1) * HG, HG)
        cidx = g % PPG
        return [
            pltpu.make_async_copy(wq_hbm.at[pl.ds(cidx * MQ, MQ), pl.ds(h0, HG), :],
                                  wq_raw.at[slot], wsems.at[slot, 0]),
            pltpu.make_async_copy(wuk_hbm.at[pl.ds(cidx * MK, MK), pl.ds(h0, HG), :],
                                  wuk_raw.at[slot], wsems.at[slot, 1]),
            pltpu.make_async_copy(wuv_hbm.at[pl.ds(cidx * MK, MK), pl.ds(h0, HG), :],
                                  wuv_raw.at[slot], wsems.at[slot, 2]),
        ]

    def wo_copy(g):
        return pltpu.make_async_copy(wo_hbm.at[g], wo_v.at[g], wsems.at[g % 2, 3])

    for c_ in cp_wmoda + cp_x:
        c_.start()
    acc_s[...] = jnp.zeros((S, M), f32)
    ctx_s[...] = jnp.zeros((S, HC * D), bf16)
    g_s[0:PAD, :] = jnp.zeros((PAD, M), f32)
    g_s[PAD + S:PAD + S + PAD, :] = jnp.zeros((PAD, M), f32)

    cv = jnp.broadcast_to(c_ref[...].astype(f32), (16, M))
    sil = (cv * jax.nn.sigmoid(cv)).astype(bf16)
    for c_ in cp_wmoda:
        c_.wait()
    cp_wq0.start()
    mod_s[:, 0:2 * M] = _mm(sil, wmod_v[:, 0:2 * M])[0:8, :]

    def mod(i):
        return mod_s[0:1, i * M:(i + 1) * M]

    sa, ca = mod(0), mod(1)
    for t, nxt in enumerate((cp_wuk0, cp_wuv0, cp_ckv[0], cp_ckv[1])):
        cp_x[t].wait()
        nxt.start()
        for r0 in range(t * XR, (t + 1) * XR, BQ):
            xr = x_v[r0:r0 + BQ, :].astype(f32)
            h_s[r0:r0 + BQ, :] = ((_ln(xr) * (1.0 + ca) + sa) * QSCALE).astype(bf16)

    for n, (cpw, raw, dst) in enumerate(((cp_wq0, wq_raw0, wq_t), (cp_wuk0, wuk_raw0, wuk_t),
                                         (cp_wuv0, wuv_raw0, wuv_t))):
        cpw.wait()
        if n == 2:
            wo_copy(0).start()
            for c_ in raw_copies(0):
                c_.start()
        t = jnp.swapaxes(raw[...], 0, 1)
        for j in range(HG):
            dst[j // HC, :, (j % HC) * D:(j % HC + 1) * D] = t[j]
    for c_ in cp_ckv:
        c_.wait()

    NRAW = NP - PPG

    def group(g, carry):
        wo_copy(g).wait()

        @pl.when(g < NRAW)
        def _():
            for c_ in raw_copies(g):
                c_.wait()

        @pl.when(g + 1 < NRAW)
        def _():
            for c_ in raw_copies(g + 1):
                c_.start()

        @pl.when(g + 1 < NP)
        def _():
            wo_copy(g + 1).start()

        for gi, c_ in enumerate((cp_wmodb, cp_w1, cp_w2, cp_w3, cp_w4)):
            pl.when(g == gi + 1)(c_.start)

        st = {}

        def pq(i):
            lo, hi = i * BQ, (i + 1) * BQ
            q_s[lo:hi, :] = _mm(h_s[lo:hi, :], wq_t[g]).astype(bf16)

        def pk(i):
            lo, hi = i * BQ, (i + 1) * BQ
            k_s[lo:hi, :] = _mm(ckv_v[lo:hi, :], wuk_t[g]).astype(bf16)

        def pv(i):
            lo, hi = i * BQ, (i + 1) * BQ
            v_s[lo:hi, :] = _mm(ckv_v[lo:hi, :], wuv_t[g]).astype(bf16)

        def po(i, gg):
            lo, hi = i * BQ, (i + 1) * BQ
            acc_s[lo:hi, :] += _mm(ctx_s[lo:hi, :], wo_v[gg])

        def nkc(i):
            return i * BQ // KC

        def qk_chunk(i, j, c):
            lo = i * BQ
            cl, ch = j * D, (j + 1) * D
            d = st.setdefault((i, j), dict(s=[], mx=None))
            if c == 0:
                d['q'] = q_s[lo:lo + BQ, cl:ch]
            q = d['q']
            if c < nkc(i):
                sc = _mm_nt(q, k_s[c * KC:(c + 1) * KC, cl:ch])
                d['s'].append(sc)
                t = functools.reduce(jnp.maximum, [sc[:, u:u + D] for u in range(0, KC, D)])
                d['mx'] = t if d['mx'] is None else jnp.maximum(d['mx'], t)
            else:
                r = jax.lax.broadcasted_iota(jnp.int32, (D, D), 0)
                cc = jax.lax.broadcasted_iota(jnp.int32, (D, D), 1)
                tri = cc <= r
                mx = d['mx']
                tiles = []
                for t in range(BQ // D):
                    st_ = _mm_nt(q[t * D:], k_s[lo + t * D:lo + (t + 1) * D, cl:ch])
                    top = jnp.where(tri, st_[:D], NEG)
                    st_ = top if t == BQ // D - 1 else jnp.concatenate([top, st_[D:]], axis=0)
                    tiles.append(st_)
                    if mx is None:
                        mx = st_
                    elif t == 0:
                        mx = jnp.maximum(mx, st_)
                    else:
                        mx = jnp.concatenate([mx[:t * D], jnp.maximum(mx[t * D:], st_)], axis=0)
                d['s'].append(tiles)
                d['m'] = jnp.max(mx, axis=1, keepdims=True)

        def epv_chunk(i, j, c):
            lo = i * BQ
            cl, ch = j * D, (j + 1) * D
            d = st[(i, j)]
            m = d['m']
            if c < nkc(i):
                sc = d['s'][c]
                ps = [jnp.exp2(sc[:, u:u + D] - m) for u in range(0, KC, D)]
                pb = jnp.concatenate([p_.astype(bf16) for p_ in ps], axis=1)
                o = _mm(pb, v_s[c * KC:(c + 1) * KC, cl:ch])
                d['acc'] = o if c == 0 else d['acc'] + o
                t = functools.reduce(jnp.add, ps)
                d['l'] = t if c == 0 else d['l'] + t
            else:
                l = d['l'] if c > 0 else None
                acc = d['acc'] if c > 0 else None
                for t, st_ in enumerate(d['s'][c]):
                    p = jnp.exp2(st_ - m[t * D:])
                    o = _mm(p.astype(bf16), v_s[lo + t * D:lo + (t + 1) * D, cl:ch])
                    if l is None:
                        l, acc = p, o
                    elif t == 0:
                        l, acc = l + p, acc + o
                    else:
                        l = jnp.concatenate([l[:t * D], l[t * D:] + p], axis=0)
                        acc = jnp.concatenate([acc[:t * D], acc[t * D:] + o], axis=0)
                lsum = jnp.sum(l, axis=1, keepdims=True)
                ctx_s[lo:lo + BQ, cl:ch] = (acc / lsum).astype(bf16)

        def phase(qk_unit, epv_unit, fillers):
            nq = nkc(qk_unit[0]) + 1 if qk_unit is not None else 0
            ne = nkc(epv_unit[0]) + 1 if epv_unit is not None else 0
            n = max(nq, ne)
            nf = len(fillers)
            fpos = [((2 * t + 1) * n) // (2 * nf) for t in range(nf)]
            for c in range(n):
                if c < nq:
                    qk_chunk(qk_unit[0], qk_unit[1], c)
                for t in range(nf):
                    if fpos[t] == c:
                        fillers[t]()
                if c < ne:
                    epv_chunk(epv_unit[0], epv_unit[1], c)

        def relayout():
            slot = g % 2
            cidx = g % PPG
            for raw, dst, mc in ((wq_raw, wq_t, MQ), (wuk_raw, wuk_t, MK), (wuv_raw, wuv_t, MK)):
                t = jnp.swapaxes(raw[slot], 0, 1)
                r0 = pl.multiple_of(cidx * mc, 16)
                for j in range(HG):
                    pidx = ((g // PPG + 1) * PPG + j) % NP
                    dst[pidx, pl.ds(r0, mc), :] = t[j]

        P = functools.partial
        pq(NB - 1)
        for c in range(LAG):
            pk(c)
        po(ORDER[-1], jnp.maximum(g - 1, 0))
        pq(NB - 2)
        R = BQ // KC
        for c in range(NB):
            if c + LAG < NB:
                pk(c + LAG)
            for cc_ in range(c * R, (c + 1) * R if c < NB - 1 else c * R + 1):
                qk_chunk(NB - 1, 0, cc_)
            pv(c)
        for n, i in enumerate(ORDER):
            f = []
            if n + 2 < NB:
                f += [P(pq, ORDER[n + 2])]
            if n >= 1:
                f += [P(po, ORDER[n - 1], g)]
            if n == TPOS:
                f += [relayout]
            phase((ORDER[n + 1], 0) if n + 1 < NB else None, (i, 0), f)
        return carry

    jax.lax.fori_loop(0, NP, group, 0)
    lo_, hi_ = ORDER[-1] * BQ, (ORDER[-1] + 1) * BQ
    acc_s[lo_:hi_, :] += _mm(ctx_s[lo_:hi_, :], wo_v[NP - 1])

    cp_wmodb.wait()
    mod_s[:, 2 * M:6 * M] = _mm(sil, wmod_v[:, 2 * M:6 * M])[0:8, :]
    ga, sb, cb, gb = mod(2), mod(3), mod(4), mod(5)
    cp_w1.wait()
    cp_w2.wait()
    cp_w3.wait()
    cp_w4.wait()
    NR = S // BM
    lane = jax.lax.broadcasted_iota(jnp.int32, (BM, 128), 1)
    cp_out = [cp(16 + r, out_v.at[r * BM:(r + 1) * BM, :], out_hbm.at[0, r * BM:(r + 1) * BM, :])
              for r in range(NR)]
    fchunks = [(lo, min(lo + FC, F)) for lo in range(0, F, FC)]
    sv = {}

    def stage1(r):
        lo, hi = r * BM, (r + 1) * BM
        x1 = x_v[lo:hi, :].astype(f32) + ga * acc_s[lo:hi, :]
        hb = _ln(x1) * (1.0 + cb) + sb
        acc_s[lo:hi, :] = x1
        hb_s[lo:hi, :] = hb
        u = _ln(hb).astype(bf16)
        g_s[PAD + lo:PAD + hi, :] = _gelu(_mm(u, w1_v[...]))

    def mix(r):
        lo, hi = r * BM, (r + 1) * BM

        def sh(d, t):
            return g_s[PAD + lo + d:PAD + hi + d, t * 128:(t + 1) * 128]

        t0 = sh(-1, 0)
        t1 = jnp.where(lane < 32, sh(-1, 1), sh(1, 1))
        t2 = jnp.where(lane < 64, sh(1, 2), sh(-2, 2))
        t3 = jnp.where(lane < 96, sh(-2, 3), sh(2, 3))
        t4 = sh(2, 4)
        gs = jnp.concatenate([t0, t1, t2, t3, t4], axis=1).astype(bf16)
        sv[r] = dict(xb=hb_s[lo:hi, :] + _mm(gs, w2_v[...]))

    def norm(r):
        sv[r]['u'] = _ln(sv[r]['xb']).astype(bf16)

    def up(r, c):
        lo, hi = fchunks[c]
        sv[r][('h', c)] = _mm_nt(sv[r]['u'], w3_v[lo:hi, :])

    def down(r, c):
        lo, hi = fchunks[c]
        o = _mm(_gelu(sv[r][('h', c)]).astype(bf16), w4_v[lo:hi, :])
        sv[r]['o'] = o if c == 0 else sv[r]['o'] + o

    def finish(r):
        lo, hi = r * BM, (r + 1) * BM
        out_v[lo:hi, :] = (acc_s[lo:hi, :] + gb * (sv[r]['xb'] + sv[r]['o'])).astype(bf16)
        cp_out[r].start()

    nc = len(fchunks)
    for r in range(min(2, NR)):
        stage1(r)
    mix(0)
    norm(0)
    for r in range(NR):
        up(r, 0)
        for c in range(nc):
            if c + 1 < nc:
                up(r, c + 1)
            if c == 0 and r + 2 < NR:
                stage1(r + 2)
            if c == 1 and r + 1 < NR:
                mix(r + 1)
            if c == 2 and r + 1 < NR:
                norm(r + 1)
            down(r, c)
        finish(r)
    for r in range(NR):
        cp_out[r].wait()


@jax.jit
def pallas_adaLN_cond__compressed_kv_cla__mixer_s_mlp__prompt_kernel(
    A_x: jax.Array,
    A_c_kv: jax.Array,
    A_w_q: jax.Array,
    A_w_uk: jax.Array,
    A_w_uv: jax.Array,
    A_w_o: jax.Array,
    B_x: jax.Array,
    B_w1: jax.Array,
    B_w2: jax.Array,
    B_w3: jax.Array,
    B_w4: jax.Array,
    c: jax.Array,
    w_mod: jax.Array,
):
    del B_x
    any_spec = pl.BlockSpec(memory_space=pltpu.HBM)
    V = pltpu.VMEM
    scratch = [
        V((S, M), bf16), V((S, DC), bf16),
        V((M, HG, D), bf16), V((DC, HG, D), bf16), V((DC, HG, D), bf16),
        V((2, M // PPG, HG, D), bf16), V((2, DC // PPG, HG, D), bf16), V((2, DC // PPG, HG, D), bf16),
        V((NP, HC * D, M), bf16),
        V((M, M), bf16), V((M, M), bf16), V((F, M), bf16), V((F, M), bf16), V((M, 6 * M), bf16),
        V((NP, M, HC * D), bf16), V((NP, DC, HC * D), bf16), V((NP, DC, HC * D), bf16),
        V((8, 6 * M), f32), V((S, M), bf16),
        V((S, HC * D), bf16), V((S, HC * D), bf16), V((S, HC * D), bf16), V((S, HC * D), bf16),
        V((S, M), f32), V((S, M), f32), V((S + 2 * PAD, M), f32), V((S, M), bf16),
        pltpu.SemaphoreType.DMA((16 + S // BM,)),
        pltpu.SemaphoreType.DMA((2, 4)),
    ]
    out = pl.pallas_call(
        _kernel,
        out_shape=jax.ShapeDtypeStruct((1, S, M), bf16),
        in_specs=[pl.BlockSpec(memory_space=pltpu.VMEM)] + [any_spec] * 11,
        out_specs=any_spec,
        scratch_shapes=scratch,
        compiler_params=pltpu.CompilerParams(vmem_limit_bytes=120 * 1024 * 1024),
    )(c, A_x.reshape(S, M), A_c_kv.reshape(S, DC), A_w_q, A_w_uk, A_w_uv, A_w_o.reshape(NP, HC * D, M),
      B_w1, B_w2, B_w3.T, B_w4, w_mod)
    return out
```

```python
import functools
import math

import jax
import jax.numpy as jnp
import jax.experimental.pallas as pl
import jax.experimental.pallas.tpu as pltpu

S = 2048
M = 640
H = 32
D = 128
DC = 4 * D
F = 1728
HG = 8
NG = H // HG
HC = 1
NP = H // HC
PPG = HG // HC
BQ = 256
NB = S // BQ
KC = 256
ORDER = (7, 6, 5, 4, 3, 2, 0, 1)
TPOS = 7
LAG = 3
BM = 128
FC = 512
PAD = 8
EPS = 1e-05
LOG2E = math.log2(math.e)
NT = (((1,), (1,)), ((), ()))
NEG = -1000000000.0 * LOG2E
QSCALE = (D ** -0.5) * LOG2E
bf16 = jnp.bfloat16
f32 = jnp.float32


def _mm(a, b):
    return jnp.dot(a, b, preferred_element_type=f32)


def _mm_nt(a, b):
    return jax.lax.dot_general(a, b, NT, preferred_element_type=f32)


def _cat(ref, lo, hi):
    return jnp.concatenate([ref[u, lo:hi, :] for u in range(ref.shape[0])], axis=1)


def _ln(x):
    m = jnp.mean(x, axis=-1, keepdims=True)
    xc = x - m
    v = jnp.mean(xc * xc, axis=-1, keepdims=True)
    return xc * jax.lax.rsqrt(v + EPS)


def _gelu(x):
    k0 = math.sqrt(2.0 / math.pi)
    return 0.5 * x * (1.0 + jnp.tanh(k0 * (x + 0.044715 * (x * x * x))))


def _kernel(c_ref, x_hbm, ckv_hbm, wq_hbm, wuk_hbm, wuv_hbm, wo_hbm,
            w1_hbm, w2_hbm, w3_hbm, w4_hbm, wmod_hbm,
            out_hbm,
            x_v, ckv_v, wq_raw0, wuk_raw0, wuv_raw0, wq_raw, wuk_raw, wuv_raw, wo_v,
            w1_v, w2_v, w3_v, w4_v, wmod_v,
            wq_t, wuk_t, wuv_t,
            mod_s, h_s, q_s, k_s, v_s, ctx_s, acc_s, hb_s, g_s, out_v, sems, wsems):
    def cp(i, src, dst):
        return pltpu.make_async_copy(src, dst, sems.at[i])

    XC = 4
    XR = S // XC
    cp_wmoda = [cp(t, wmod_hbm.at[t * (M // 2):(t + 1) * (M // 2), 0:2 * M],
                   wmod_v.at[t * (M // 2):(t + 1) * (M // 2), 0:2 * M]) for t in range(2)]
    cp_x = [cp(2 + t, x_hbm.at[t * XR:(t + 1) * XR, :], x_v.at[t * XR:(t + 1) * XR, :])
            for t in range(XC)]
    cp_ckv = [cp(6 + t, ckv_hbm.at[t * (S // 2):(t + 1) * (S // 2), :],
                 ckv_v.at[t * (S // 2):(t + 1) * (S // 2), :]) for t in range(2)]
    cp_wuk0 = cp(8, wuk_hbm.at[:, 0:HG, :], wuk_raw0)
    cp_wuv0 = cp(9, wuv_hbm.at[:, 0:HG, :], wuv_raw0)
    cp_wq0 = cp(10, wq_hbm.at[:, 0:HG, :], wq_raw0)
    cp_wmodb = cp(11, wmod_hbm.at[:, 2 * M:6 * M], wmod_v.at[:, 2 * M:6 * M])
    cp_w1 = cp(12, w1_hbm, w1_v)
    cp_w2 = cp(13, w2_hbm, w2_v)
    cp_w3 = cp(14, w3_hbm, w3_v)
    cp_w4 = cp(15, w4_hbm, w4_v)

    MQ, MK = M // PPG, DC // PPG

    def raw_copies(g):
        slot = g % 2
        h0 = pl.multiple_of((g // PPG + 1) * HG, HG)
        cidx = g % PPG
        return [
            pltpu.make_async_copy(src.at[pl.ds(cidx * mc, mc), pl.ds(h0, HG), :],
                                  raw.at[slot], wsems.at[slot, n])
            for n, (src, raw, mc) in enumerate(((wq_hbm, wq_raw, MQ), (wuk_hbm, wuk_raw, MK),
                                                (wuv_hbm, wuv_raw, MK)))]

    def wo_copy(g):
        return pltpu.make_async_copy(wo_hbm.at[g], wo_v.at[g], wsems.at[g % 2, 3])

    for c_ in [cp_wuk0] + cp_ckv + [cp_wuv0]:
        c_.start()
    g_s[0:PAD, :] = jnp.zeros((PAD, M), f32)
    g_s[PAD + S:PAD + S + PAD, :] = jnp.zeros((PAD, M), f32)
    cv = jnp.broadcast_to(c_ref[...].astype(f32), (16, M))
    sil = (cv * jax.nn.sigmoid(cv)).astype(bf16)

    def relayout0(raw, dst):
        t = jnp.swapaxes(raw[...], 0, 1)
        for j in range(HG):
            dst[j] = t[j]

    cp_wuk0.wait()
    for c_ in cp_wmoda:
        c_.start()
    relayout0(wuk_raw0, wuk_t)
    for c_ in cp_ckv:
        c_.wait()
    for c_ in cp_x:
        c_.start()
    for r in range(NB):
        lo, hi = r * BQ, (r + 1) * BQ
        k_s[lo:hi, :] = _mm(ckv_v[lo:hi, :], wuk_t[0]).astype(bf16)
    cp_wuv0.wait()
    cp_wq0.start()
    relayout0(wuv_raw0, wuv_t)
    for r in range(NB):
        lo, hi = r * BQ, (r + 1) * BQ
        v_s[lo:hi, :] = _mm(ckv_v[lo:hi, :], wuv_t[0]).astype(bf16)

    for c_ in cp_wmoda:
        c_.wait()
    wo_copy(0).start()
    for c_ in raw_copies(0):
        c_.start()
    mod_s[:, 0:2 * M] = _mm(sil, wmod_v[:, 0:2 * M])[0:8, :]

    def mod(i):
        return mod_s[0:1, i * M:(i + 1) * M]

    sa, ca = mod(0), mod(1)
    for t in range(XC):
        cp_x[t].wait()
        for r0 in range(t * XR, (t + 1) * XR, BQ):
            xr = x_v[r0:r0 + BQ, :].astype(f32)
            hr = ((_ln(xr) * (1.0 + ca) + sa) * QSCALE).astype(bf16)
            for u in range(M // D):
                h_s[u, r0:r0 + BQ, :] = hr[:, u * D:(u + 1) * D]
    cp_wq0.wait()
    relayout0(wq_raw0, wq_t)


    NRAW = NP - PPG

    def head(g, first):
        wo_copy(g).wait()
        def when(cond, fn):
            if first:
                if cond:
                    fn()
            else:
                pl.when(cond)(fn)

        def raw_wait():
            for c_ in raw_copies(g):
                c_.wait()

        def raw_start():
            for c_ in raw_copies(g + 1):
                c_.start()

        when(g < NRAW, raw_wait)
        when(g + 1 < NRAW, raw_start)
        when(g + 1 < NP, wo_copy(g + 1).start)
        for gi, c_ in enumerate((cp_wmodb, cp_w1, cp_w2, cp_w3, cp_w4)):
            when(g == gi + 1, c_.start)

        st = {}

        def pq(i):
            lo, hi = i * BQ, (i + 1) * BQ
            q_s[lo:hi, :] = _mm(_cat(h_s, lo, hi), wq_t[g]).astype(bf16)

        def pk(i):
            lo, hi = i * BQ, (i + 1) * BQ
            k_s[lo:hi, :] = _mm(ckv_v[lo:hi, :], wuk_t[g]).astype(bf16)

        def pv(i):
            lo, hi = i * BQ, (i + 1) * BQ
            v_s[lo:hi, :] = _mm(ckv_v[lo:hi, :], wuv_t[g]).astype(bf16)

        def po(i, gg):
            lo, hi = i * BQ, (i + 1) * BQ
            if first:
                acc_s[lo:hi, :] = _mm(ctx_s[lo:hi, :], wo_v[gg])
            else:
                acc_s[lo:hi, :] += _mm(ctx_s[lo:hi, :], wo_v[gg])

        def nkc(i):
            return i * BQ // KC

        def qk_chunk(i, j, c):
            lo = i * BQ
            cl, ch = j * D, (j + 1) * D
            d = st.setdefault((i, j), dict(s=[], mx=None))
            if c == 0:
                d['q'] = q_s[lo:lo + BQ, cl:ch]
            q = d['q']
            if c < nkc(i):
                sc = _mm_nt(q, k_s[c * KC:(c + 1) * KC, cl:ch])
                d['s'].append(sc)
                t = functools.reduce(jnp.maximum, [sc[:, u:u + D] for u in range(0, KC, D)])
                d['mx'] = t if d['mx'] is None else jnp.maximum(d['mx'], t)
            else:
                r = jax.lax.broadcasted_iota(jnp.int32, (D, D), 0)
                cc = jax.lax.broadcasted_iota(jnp.int32, (D, D), 1)
                tri = cc <= r
                mx = d['mx']
                tiles = []
                for t in range(BQ // D):
                    st_ = _mm_nt(q[t * D:], k_s[lo + t * D:lo + (t + 1) * D, cl:ch])
                    top = jnp.where(tri, st_[:D], NEG)
                    st_ = top if t == BQ // D - 1 else jnp.concatenate([top, st_[D:]], axis=0)
                    tiles.append(st_)
                    if mx is None:
                        mx = st_
                    elif t == 0:
                        mx = jnp.maximum(mx, st_)
                    else:
                        mx = jnp.concatenate([mx[:t * D], jnp.maximum(mx[t * D:], st_)], axis=0)
                d['s'].append(tiles)
                d['m'] = jnp.max(mx, axis=1, keepdims=True)

        def epv_chunk(i, j, c):
            lo = i * BQ
            cl, ch = j * D, (j + 1) * D
            d = st[(i, j)]
            m = d['m']
            if c < nkc(i):
                sc = d['s'][c]
                ps = [jnp.exp2(sc[:, u:u + D] - m) for u in range(0, KC, D)]
                pb = jnp.concatenate([p_.astype(bf16) for p_ in ps], axis=1)
                o = _mm(pb, v_s[c * KC:(c + 1) * KC, cl:ch])
                d['acc'] = o if c == 0 else d['acc'] + o
                t = functools.reduce(jnp.add, ps)
                d['l'] = t if c == 0 else d['l'] + t
            else:
                l = d['l'] if c > 0 else None
                acc = d['acc'] if c > 0 else None
                for t, st_ in enumerate(d['s'][c]):
                    p = jnp.exp2(st_ - m[t * D:])
                    o = _mm(p.astype(bf16), v_s[lo + t * D:lo + (t + 1) * D, cl:ch])
                    if l is None:
                        l, acc = p, o
                    elif t == 0:
                        l, acc = l + p, acc + o
                    else:
                        l = jnp.concatenate([l[:t * D], l[t * D:] + p], axis=0)
                        acc = jnp.concatenate([acc[:t * D], acc[t * D:] + o], axis=0)
                lsum = jnp.sum(l, axis=1, keepdims=True)
                ctx_s[lo:lo + BQ, cl:ch] = (acc / lsum).astype(bf16)

        def phase(qk_unit, epv_unit, fillers):
            nq = nkc(qk_unit[0]) + 1 if qk_unit is not None else 0
            ne = nkc(epv_unit[0]) + 1 if epv_unit is not None else 0
            n = max(nq, ne)
            nf = len(fillers)
            fpos = [((2 * t + 1) * n) // (2 * nf) for t in range(nf)]
            for c in range(n):
                if c < nq:
                    qk_chunk(qk_unit[0], qk_unit[1], c)
                for t in range(nf):
                    if fpos[t] == c:
                        fillers[t]()
                if c < ne:
                    epv_chunk(epv_unit[0], epv_unit[1], c)

        def relayout():
            slot = g % 2
            cidx = g % PPG
            for raw, dst, mc in ((wq_raw, wq_t, MQ), (wuk_raw, wuk_t, MK), (wuv_raw, wuv_t, MK)):
                t = jnp.swapaxes(raw[slot], 0, 1)
                r0 = pl.multiple_of(cidx * mc, 16)
                for j in range(HG):
                    pidx = ((g // PPG + 1) * PPG + j) % NP
                    dst[pidx, pl.ds(r0, mc), :] = t[j]

        P = functools.partial
        pq(NB - 1)
        if not first:
            for c in range(LAG):
                pk(c)
            po(ORDER[-1], g - 1)
        pq(NB - 2)
        R = BQ // KC
        for c in range(NB):
            if c + LAG < NB and not first:
                pk(c + LAG)
            for cc_ in range(c * R, (c + 1) * R if c < NB - 1 else c * R + 1):
                qk_chunk(NB - 1, 0, cc_)
            if not first:
                pv(c)
        for n, i in enumerate(ORDER):
            f = []
            if n + 2 < NB:
                f += [P(pq, ORDER[n + 2])]
            if n >= 1:
                f += [P(po, ORDER[n - 1], g)]
            if n == TPOS:
                f += [relayout]
            phase((ORDER[n + 1], 0) if n + 1 < NB else None, (i, 0), f)

    head(0, True)
    acc_s[ORDER[-1] * BQ:(ORDER[-1] + 1) * BQ, :] = jnp.zeros((BQ, M), f32)

    def body(g, carry):
        head(g, False)
        return carry

    jax.lax.fori_loop(1, NP, body, 0)
    lo_, hi_ = ORDER[-1] * BQ, (ORDER[-1] + 1) * BQ
    acc_s[lo_:hi_, :] += _mm(ctx_s[lo_:hi_, :], wo_v[NP - 1])

    cp_wmodb.wait()
    mod_s[:, 2 * M:6 * M] = _mm(sil, wmod_v[:, 2 * M:6 * M])[0:8, :]
    ga, sb, cb, gb = mod(2), mod(3), mod(4), mod(5)
    cp_w1.wait()
    cp_w2.wait()
    cp_w3.wait()
    cp_w4.wait()
    NR = S // BM
    lane = jax.lax.broadcasted_iota(jnp.int32, (BM, 128), 1)
    cp_out = [cp(16 + r, out_v.at[r * BM:(r + 1) * BM, :], out_hbm.at[0, r * BM:(r + 1) * BM, :])
              for r in range(NR)]
    fchunks = [(lo, min(lo + FC, F)) for lo in range(0, F, FC)]
    sv = {}

    def stage1(r):
        lo, hi = r * BM, (r + 1) * BM
        x1 = x_v[lo:hi, :].astype(f32) + ga * acc_s[lo:hi, :]
        hb = _ln(x1) * (1.0 + cb) + sb
        acc_s[lo:hi, :] = x1
        hb_s[lo:hi, :] = hb
        u = _ln(hb).astype(bf16)
        g_s[PAD + lo:PAD + hi, :] = _gelu(_mm(u, w1_v[...]))

    def mix(r):
        lo, hi = r * BM, (r + 1) * BM

        def sh(d, t):
            return g_s[PAD + lo + d:PAD + hi + d, t * 128:(t + 1) * 128]

        t0 = sh(-1, 0)
        t1 = jnp.where(lane < 32, sh(-1, 1), sh(1, 1))
        t2 = jnp.where(lane < 64, sh(1, 2), sh(-2, 2))
        t3 = jnp.where(lane < 96, sh(-2, 3), sh(2, 3))
        t4 = sh(2, 4)
        gs = jnp.concatenate([t0, t1, t2, t3, t4], axis=1).astype(bf16)
        sv[r] = dict(xb=hb_s[lo:hi, :] + _mm(gs, w2_v[...]))

    def norm(r):
        sv[r]['u'] = _ln(sv[r]['xb']).astype(bf16)

    def up(r, c):
        lo, hi = fchunks[c]
        sv[r][('h', c)] = _mm_nt(sv[r]['u'], w3_v[lo:hi, :])

    def down(r, c):
        lo, hi = fchunks[c]
        o = _mm(_gelu(sv[r][('h', c)]).astype(bf16), w4_v[lo:hi, :])
        sv[r]['o'] = o if c == 0 else sv[r]['o'] + o

    def finish(r):
        lo, hi = r * BM, (r + 1) * BM
        out_v[lo:hi, :] = (acc_s[lo:hi, :] + gb * (sv[r]['xb'] + sv[r]['o'])).astype(bf16)
        cp_out[r].start()

    nc = len(fchunks)
    for r in range(min(2, NR)):
        stage1(r)
    mix(0)
    norm(0)
    for r in range(NR):
        up(r, 0)
        for c in range(nc):
            if c + 1 < nc:
                up(r, c + 1)
            if c == 0 and r + 2 < NR:
                stage1(r + 2)
            if c == 1 and r + 1 < NR:
                mix(r + 1)
            if c == 2 and r + 1 < NR:
                norm(r + 1)
            down(r, c)
        finish(r)
    for r in range(NR):
        cp_out[r].wait()


@jax.jit
def pallas_adaLN_cond__compressed_kv_cla__mixer_s_mlp__prompt_kernel(
    A_x: jax.Array,
    A_c_kv: jax.Array,
    A_w_q: jax.Array,
    A_w_uk: jax.Array,
    A_w_uv: jax.Array,
    A_w_o: jax.Array,
    B_x: jax.Array,
    B_w1: jax.Array,
    B_w2: jax.Array,
    B_w3: jax.Array,
    B_w4: jax.Array,
    c: jax.Array,
    w_mod: jax.Array,
):
    del B_x
    any_spec = pl.BlockSpec(memory_space=pltpu.HBM)
    V = pltpu.VMEM
    scratch = [
        V((S, M), bf16), V((S, DC), bf16),
        V((M, HG, D), bf16), V((DC, HG, D), bf16), V((DC, HG, D), bf16),
        V((2, M // PPG, HG, D), bf16), V((2, DC // PPG, HG, D), bf16), V((2, DC // PPG, HG, D), bf16),
        V((NP, HC * D, M), bf16),
        V((M, M), bf16), V((M, M), bf16), V((F, M), bf16), V((F, M), bf16), V((M, 6 * M), bf16),
        V((NP, M, HC * D), bf16), V((NP, DC, HC * D), bf16), V((NP, DC, HC * D), bf16),
        V((8, 6 * M), f32), V((M // D, S, D), bf16),
        V((S, HC * D), bf16), V((S, HC * D), bf16), V((S, HC * D), bf16), V((S, HC * D), bf16),
        V((S, M), f32), V((S, M), f32), V((S + 2 * PAD, M), f32), V((S, M), bf16),
        pltpu.SemaphoreType.DMA((16 + S // BM,)),
        pltpu.SemaphoreType.DMA((2, 4)),
    ]
    out = pl.pallas_call(
        _kernel,
        out_shape=jax.ShapeDtypeStruct((1, S, M), bf16),
        in_specs=[pl.BlockSpec(memory_space=pltpu.VMEM)] + [any_spec] * 11,
        out_specs=any_spec,
        scratch_shapes=scratch,
        compiler_params=pltpu.CompilerParams(vmem_limit_bytes=120 * 1024 * 1024),
    )(c, A_x.reshape(S, M), A_c_kv.reshape(S, DC), A_w_q, A_w_uk, A_w_uv, A_w_o.reshape(NP, HC * D, M),
      B_w1, B_w2, B_w3.T, B_w4, w_mod)
    return out
```

```python
import functools
import math

import jax
import jax.numpy as jnp
import jax.experimental.pallas as pl
import jax.experimental.pallas.tpu as pltpu

S = 2048
M = 640
H = 32
D = 128
DC = 4 * D
F = 1728
HG = 8
NG = H // HG
HC = 1
NP = H // HC
PPG = HG // HC
BQ = 256
NB = S // BQ
KC = 256
ORDER = (7, 6, 5, 4, 3, 2, 0, 1)
TPOS = 7
LAG = 3
BM = 128
FC = 512
PAD = 8
EPS = 1e-05
LOG2E = math.log2(math.e)
NT = (((1,), (1,)), ((), ()))
NEG = -1000000000.0 * LOG2E
QSCALE = (D ** -0.5) * LOG2E
bf16 = jnp.bfloat16
f32 = jnp.float32


def _mm(a, b):
    return jnp.dot(a, b, preferred_element_type=f32)


def _mm_nt(a, b):
    return jax.lax.dot_general(a, b, NT, preferred_element_type=f32)


def _cat(ref, lo, hi):
    return jnp.concatenate([ref[u, lo:hi, :] for u in range(ref.shape[0])], axis=1)


def _ln(x):
    m = jnp.mean(x, axis=-1, keepdims=True)
    xc = x - m
    v = jnp.mean(xc * xc, axis=-1, keepdims=True)
    return xc * jax.lax.rsqrt(v + EPS)


def _gelu(x):
    k0 = math.sqrt(2.0 / math.pi)
    return 0.5 * x * (1.0 + jnp.tanh(k0 * (x + 0.044715 * (x * x * x))))


def _kernel(c_ref, x_hbm, ckv_hbm, wq_hbm, wuk_hbm, wuv_hbm, wo_hbm,
            w1_hbm, w2_hbm, w3_hbm, w4_hbm, wmod_hbm,
            out_hbm,
            x_v, ckv_v, wq_raw0, wuk_raw0, wuv_raw0, wq_raw, wuk_raw, wuv_raw, wo_v,
            w1_v, w2_v, w3_v, w4_v, wmod_v,
            wq_t, wuk_t, wuv_t,
            mod_s, h_s, q_s, k_s, v_s, ctx_s, acc_s, hb_s, g_s, out_v, sems, wsems):
    def cp(i, src, dst):
        return pltpu.make_async_copy(src, dst, sems.at[i])

    XC = 4
    XR = S // XC
    cp_wmoda = [cp(t, wmod_hbm.at[t * (M // 2):(t + 1) * (M // 2), 0:2 * M],
                   wmod_v.at[t * (M // 2):(t + 1) * (M // 2), 0:2 * M]) for t in range(2)]
    cp_x = [cp(2 + t, x_hbm.at[t * XR:(t + 1) * XR, :], x_v.at[t * XR:(t + 1) * XR, :])
            for t in range(XC)]
    cp_ckv = [cp(6 + t, ckv_hbm.at[t * (S // 2):(t + 1) * (S // 2), :],
                 ckv_v.at[t * (S // 2):(t + 1) * (S // 2), :]) for t in range(2)]
    cp_wuk0 = cp(8, wuk_hbm.at[:, 0:HG, :], wuk_raw0)
    cp_wuv0 = cp(9, wuv_hbm.at[:, 0:HG, :], wuv_raw0)
    cp_wq0 = cp(10, wq_hbm.at[:, 0:HG, :], wq_raw0)
    cp_wmodb = cp(11, wmod_hbm.at[:, 2 * M:6 * M], wmod_v.at[:, 2 * M:6 * M])
    cp_w1 = cp(12, w1_hbm, w1_v)
    cp_w2 = cp(13, w2_hbm, w2_v)
    cp_w3 = cp(14, w3_hbm, w3_v)
    cp_w4 = cp(15, w4_hbm, w4_v)

    MQ, MK = M // PPG, DC // PPG

    def raw_copies(g):
        slot = g % 2
        h0 = pl.multiple_of((g // PPG + 1) * HG, HG)
        cidx = g % PPG
        return [
            pltpu.make_async_copy(src.at[pl.ds(cidx * mc, mc), pl.ds(h0, HG), :],
                                  raw.at[slot], wsems.at[slot, n])
            for n, (src, raw, mc) in enumerate(((wq_hbm, wq_raw, MQ), (wuk_hbm, wuk_raw, MK),
                                                (wuv_hbm, wuv_raw, MK)))]

    def wo_copy(g):
        return pltpu.make_async_copy(wo_hbm.at[g], wo_v.at[g], wsems.at[g % 2, 3])

    for c_ in [cp_wuk0] + cp_ckv + [cp_wuv0]:
        c_.start()
    g_s[0:PAD, :] = jnp.zeros((PAD, M), f32)
    g_s[PAD + S:PAD + S + PAD, :] = jnp.zeros((PAD, M), f32)
    cv = jnp.broadcast_to(c_ref[...].astype(f32), (16, M))
    sil = (cv * jax.nn.sigmoid(cv)).astype(bf16)

    def relayout0(raw, dst):
        t = jnp.swapaxes(raw[...], 0, 1)
        for j in range(HG):
            dst[j] = t[j]

    cp_wuk0.wait()
    for c_ in cp_wmoda:
        c_.start()
    relayout0(wuk_raw0, wuk_t)
    for c_ in cp_ckv:
        c_.wait()
    cp_x[XC - 1].start()
    cp_wq0.start()
    for r in range(NB):
        lo, hi = r * BQ, (r + 1) * BQ
        k_s[lo:hi, :] = _mm(ckv_v[lo:hi, :], wuk_t[0]).astype(bf16)
    cp_wuv0.wait()
    wo_copy(0).start()
    cp_x[XC - 2].start()
    relayout0(wuv_raw0, wuv_t)
    for r in range(NB):
        lo, hi = r * BQ, (r + 1) * BQ
        v_s[lo:hi, :] = _mm(ckv_v[lo:hi, :], wuv_t[0]).astype(bf16)

    for c_ in cp_wmoda:
        c_.wait()
    for c_ in raw_copies(0) + cp_x[:XC - 2][::-1]:
        c_.start()
    mod_s[:, 0:2 * M] = _mm(sil, wmod_v[:, 0:2 * M])[0:8, :]

    def mod(i):
        return mod_s[0:1, i * M:(i + 1) * M]

    def norm_x(t):
        sa, ca = mod(0) * QSCALE, (1.0 + mod(1)) * QSCALE
        cp_x[t].wait()
        for r0 in range(t * XR, (t + 1) * XR, BQ):
            xr = x_v[r0:r0 + BQ, :].astype(f32)
            hr = (_ln(xr) * ca + sa).astype(bf16)
            for u in range(M // D):
                h_s[u, r0:r0 + BQ, :] = hr[:, u * D:(u + 1) * D]

    norm_x(XC - 1)
    cp_wq0.wait()
    relayout0(wq_raw0, wq_t)


    NRAW = NP - PPG

    def head(g, first):
        if not first:
            wo_copy(g).wait()
        def when(cond, fn):
            if first:
                if cond:
                    fn()
            else:
                pl.when(cond)(fn)

        def raw_wait():
            for c_ in raw_copies(g):
                c_.wait()

        def raw_start():
            for c_ in raw_copies(g + 1):
                c_.start()

        if not first:
            when(g < NRAW, raw_wait)
            when(g + 1 < NRAW, raw_start)
            when(g + 1 < NP, wo_copy(g + 1).start)
        for gi, c_ in enumerate((cp_wmodb, cp_w1, cp_w2, cp_w3, cp_w4)):
            when(g == gi + 1, c_.start)

        st = {}

        def pq(i):
            lo, hi = i * BQ, (i + 1) * BQ
            q_s[lo:hi, :] = _mm(_cat(h_s, lo, hi), wq_t[g]).astype(bf16)

        def pk(i):
            lo, hi = i * BQ, (i + 1) * BQ
            k_s[lo:hi, :] = _mm(ckv_v[lo:hi, :], wuk_t[g]).astype(bf16)

        def pv(i):
            lo, hi = i * BQ, (i + 1) * BQ
            v_s[lo:hi, :] = _mm(ckv_v[lo:hi, :], wuv_t[g]).astype(bf16)

        def po(i, gg):
            lo, hi = i * BQ, (i + 1) * BQ
            if first:
                acc_s[lo:hi, :] = _mm(ctx_s[lo:hi, :], wo_v[gg])
            else:
                acc_s[lo:hi, :] += _mm(ctx_s[lo:hi, :], wo_v[gg])

        def nkc(i):
            return i * BQ // KC

        def qk_chunk(i, j, c):
            lo = i * BQ
            cl, ch = j * D, (j + 1) * D
            d = st.setdefault((i, j), dict(s=[], mx=None))
            if c == 0:
                d['q'] = q_s[lo:lo + BQ, cl:ch]
            q = d['q']
            if c < nkc(i):
                sc = _mm_nt(q, k_s[c * KC:(c + 1) * KC, cl:ch])
                d['s'].append(sc)
                t = functools.reduce(jnp.maximum, [sc[:, u:u + D] for u in range(0, KC, D)])
                d['mx'] = t if d['mx'] is None else jnp.maximum(d['mx'], t)
            else:
                r = jax.lax.broadcasted_iota(jnp.int32, (D, D), 0)
                cc = jax.lax.broadcasted_iota(jnp.int32, (D, D), 1)
                tri = cc <= r
                mx = d['mx']
                tiles = []
                for t in range(BQ // D):
                    st_ = _mm_nt(q[t * D:], k_s[lo + t * D:lo + (t + 1) * D, cl:ch])
                    top = jnp.where(tri, st_[:D], NEG)
                    st_ = top if t == BQ // D - 1 else jnp.concatenate([top, st_[D:]], axis=0)
                    tiles.append(st_)
                    if mx is None:
                        mx = st_
                    elif t == 0:
                        mx = jnp.maximum(mx, st_)
                    else:
                        mx = jnp.concatenate([mx[:t * D], jnp.maximum(mx[t * D:], st_)], axis=0)
                d['s'].append(tiles)
                d['m'] = jnp.max(mx, axis=1, keepdims=True)

        def epv_chunk(i, j, c):
            lo = i * BQ
            cl, ch = j * D, (j + 1) * D
            d = st[(i, j)]
            m = d['m']
            if c < nkc(i):
                sc = d['s'][c]
                ps = [jnp.exp2(sc[:, u:u + D] - m) for u in range(0, KC, D)]
                pb = jnp.concatenate([p_.astype(bf16) for p_ in ps], axis=1)
                o = _mm(pb, v_s[c * KC:(c + 1) * KC, cl:ch])
                d['acc'] = o if c == 0 else d['acc'] + o
                t = functools.reduce(jnp.add, ps)
                d['l'] = t if c == 0 else d['l'] + t
            else:
                l = d['l'] if c > 0 else None
                acc = d['acc'] if c > 0 else None
                for t, st_ in enumerate(d['s'][c]):
                    p = jnp.exp2(st_ - m[t * D:])
                    o = _mm(p.astype(bf16), v_s[lo + t * D:lo + (t + 1) * D, cl:ch])
                    if l is None:
                        l, acc = p, o
                    elif t == 0:
                        l, acc = l + p, acc + o
                    else:
                        l = jnp.concatenate([l[:t * D], l[t * D:] + p], axis=0)
                        acc = jnp.concatenate([acc[:t * D], acc[t * D:] + o], axis=0)
                lsum = jnp.sum(l, axis=1, keepdims=True)
                ctx_s[lo:lo + BQ, cl:ch] = (acc / lsum).astype(bf16)

        def phase(qk_unit, epv_unit, fillers):
            nq = nkc(qk_unit[0]) + 1 if qk_unit is not None else 0
            ne = nkc(epv_unit[0]) + 1 if epv_unit is not None else 0
            n = max(nq, ne)
            nf = len(fillers)
            fpos = [((2 * t + 1) * n) // (2 * nf) for t in range(nf)]
            for c in range(n):
                if c < nq:
                    qk_chunk(qk_unit[0], qk_unit[1], c)
                for t in range(nf):
                    if fpos[t] == c:
                        fillers[t]()
                if c < ne:
                    epv_chunk(epv_unit[0], epv_unit[1], c)

        def relayout():
            slot = g % 2
            cidx = g % PPG
            for raw, dst, mc in ((wq_raw, wq_t, MQ), (wuk_raw, wuk_t, MK), (wuv_raw, wuv_t, MK)):
                t = jnp.swapaxes(raw[slot], 0, 1)
                r0 = pl.multiple_of(cidx * mc, 16)
                for j in range(HG):
                    pidx = ((g // PPG + 1) * PPG + j) % NP
                    dst[pidx, pl.ds(r0, mc), :] = t[j]

        P = functools.partial
        pq(NB - 1)
        if not first:
            for c in range(LAG):
                pk(c)
            po(ORDER[-1], g - 1)
        pq(NB - 2)
        R = BQ // KC
        for c in range(NB):
            if c + LAG < NB and not first:
                pk(c + LAG)
            for cc_ in range(c * R, (c + 1) * R if c < NB - 1 else c * R + 1):
                qk_chunk(NB - 1, 0, cc_)
            if not first:
                pv(c)
        for n, i in enumerate(ORDER):
            if first:
                if n == 0:
                    wo_copy(0).wait()
                if n + 2 < NB and n % 2 == 0:
                    norm_x(XC - 2 - n // 2)
                if n == 2:
                    raw_start()
                    wo_copy(1).start()
                if n == TPOS:
                    raw_wait()
            f = []
            if n + 2 < NB:
                f += [P(pq, ORDER[n + 2])]
            if n >= 1:
                f += [P(po, ORDER[n - 1], g)]
            if n == TPOS:
                f += [relayout]
            phase((ORDER[n + 1], 0) if n + 1 < NB else None, (i, 0), f)

    head(0, True)
    acc_s[ORDER[-1] * BQ:(ORDER[-1] + 1) * BQ, :] = jnp.zeros((BQ, M), f32)

    def body(g, carry):
        head(g, False)
        return carry

    jax.lax.fori_loop(1, NP, body, 0)
    lo_, hi_ = ORDER[-1] * BQ, (ORDER[-1] + 1) * BQ
    acc_s[lo_:hi_, :] += _mm(ctx_s[lo_:hi_, :], wo_v[NP - 1])

    cp_wmodb.wait()
    mod_s[:, 2 * M:6 * M] = _mm(sil, wmod_v[:, 2 * M:6 * M])[0:8, :]
    ga, sb, cb, gb = mod(2), mod(3), mod(4), mod(5)
    cp_w1.wait()
    cp_w2.wait()
    cp_w3.wait()
    cp_w4.wait()
    NR = S // BM
    lane = jax.lax.broadcasted_iota(jnp.int32, (BM, 128), 1)
    cp_out = [cp(16 + r, out_v.at[r * BM:(r + 1) * BM, :], out_hbm.at[0, r * BM:(r + 1) * BM, :])
              for r in range(NR)]
    fchunks = [(lo, min(lo + FC, F)) for lo in range(0, F, FC)]
    sv = {}

    def stage1(r):
        lo, hi = r * BM, (r + 1) * BM
        x1 = x_v[lo:hi, :].astype(f32) + ga * acc_s[lo:hi, :]
        hb = _ln(x1) * (1.0 + cb) + sb
        acc_s[lo:hi, :] = x1
        hb_s[lo:hi, :] = hb
        u = _ln(hb).astype(bf16)
        g_s[PAD + lo:PAD + hi, :] = _gelu(_mm(u, w1_v[...]))

    def mix(r):
        lo, hi = r * BM, (r + 1) * BM

        def sh(d, t):
            return g_s[PAD + lo + d:PAD + hi + d, t * 128:(t + 1) * 128]

        t0 = sh(-1, 0)
        t1 = jnp.where(lane < 32, sh(-1, 1), sh(1, 1))
        t2 = jnp.where(lane < 64, sh(1, 2), sh(-2, 2))
        t3 = jnp.where(lane < 96, sh(-2, 3), sh(2, 3))
        t4 = sh(2, 4)
        gs = jnp.concatenate([t0, t1, t2, t3, t4], axis=1).astype(bf16)
        sv[r] = dict(xb=hb_s[lo:hi, :] + _mm(gs, w2_v[...]))

    def norm(r):
        sv[r]['u'] = _ln(sv[r]['xb']).astype(bf16)

    def up(r, c):
        lo, hi = fchunks[c]
        sv[r][('h', c)] = _mm_nt(sv[r]['u'], w3_v[lo:hi, :])

    def down(r, c):
        lo, hi = fchunks[c]
        o = _mm(_gelu(sv[r][('h', c)]).astype(bf16), w4_v[lo:hi, :])
        sv[r]['o'] = o if c == 0 else sv[r]['o'] + o

    def finish(r):
        lo, hi = r * BM, (r + 1) * BM
        out_v[lo:hi, :] = (acc_s[lo:hi, :] + gb * (sv[r]['xb'] + sv[r]['o'])).astype(bf16)
        cp_out[r].start()

    nc = len(fchunks)
    for r in range(min(2, NR)):
        stage1(r)
    mix(0)
    norm(0)
    for r in range(NR):
        up(r, 0)
        for c in range(nc):
            if c + 1 < nc:
                up(r, c + 1)
            if c == 0 and r + 2 < NR:
                stage1(r + 2)
            if c == 1 and r + 1 < NR:
                mix(r + 1)
            if c == 2 and r + 1 < NR:
                norm(r + 1)
            down(r, c)
        finish(r)
    for r in range(NR):
        cp_out[r].wait()


@jax.jit
def pallas_adaLN_cond__compressed_kv_cla__mixer_s_mlp__prompt_kernel(
    A_x: jax.Array,
    A_c_kv: jax.Array,
    A_w_q: jax.Array,
    A_w_uk: jax.Array,
    A_w_uv: jax.Array,
    A_w_o: jax.Array,
    B_x: jax.Array,
    B_w1: jax.Array,
    B_w2: jax.Array,
    B_w3: jax.Array,
    B_w4: jax.Array,
    c: jax.Array,
    w_mod: jax.Array,
):
    del B_x
    any_spec = pl.BlockSpec(memory_space=pltpu.HBM)
    V = pltpu.VMEM
    scratch = [
        V((S, M), bf16), V((S, DC), bf16),
        V((M, HG, D), bf16), V((DC, HG, D), bf16), V((DC, HG, D), bf16),
        V((2, M // PPG, HG, D), bf16), V((2, DC // PPG, HG, D), bf16), V((2, DC // PPG, HG, D), bf16),
        V((NP, HC * D, M), bf16),
        V((M, M), bf16), V((M, M), bf16), V((F, M), bf16), V((F, M), bf16), V((M, 6 * M), bf16),
        V((NP, M, HC * D), bf16), V((NP, DC, HC * D), bf16), V((NP, DC, HC * D), bf16),
        V((8, 6 * M), f32), V((M // D, S, D), bf16),
        V((S, HC * D), bf16), V((S, HC * D), bf16), V((S, HC * D), bf16), V((S, HC * D), bf16),
        V((S, M), f32), V((S, M), f32), V((S + 2 * PAD, M), f32), V((S, M), bf16),
        pltpu.SemaphoreType.DMA((16 + S // BM,)),
        pltpu.SemaphoreType.DMA((2, 4)),
    ]
    out = pl.pallas_call(
        _kernel,
        out_shape=jax.ShapeDtypeStruct((1, S, M), bf16),
        in_specs=[pl.BlockSpec(memory_space=pltpu.VMEM)] + [any_spec] * 11,
        out_specs=any_spec,
        scratch_shapes=scratch,
        compiler_params=pltpu.CompilerParams(vmem_limit_bytes=120 * 1024 * 1024),
    )(c, A_x.reshape(S, M), A_c_kv.reshape(S, DC), A_w_q, A_w_uk, A_w_uv, A_w_o.reshape(NP, HC * D, M),
      B_w1, B_w2, B_w3.T, B_w4, w_mod)
    return out
```

```python
import functools
import math

import jax
import jax.numpy as jnp
import jax.experimental.pallas as pl
import jax.experimental.pallas.tpu as pltpu

S = 2048
M = 640
H = 32
D = 128
DC = 4 * D
F = 1728
HG = 8
NG = H // HG
HC = 1
NP = H // HC
PPG = HG // HC
BQ = 256
NB = S // BQ
KC = 256
ORDER = (7, 6, 5, 4, 3, 2, 0, 1)
TPOS = 7
LAG = 3
BM = 128
FC = 512
PAD = 8
EPS = 1e-05
LOG2E = math.log2(math.e)
NT = (((1,), (1,)), ((), ()))
NEG = -1000000000.0 * LOG2E
QSCALE = (D ** -0.5) * LOG2E
bf16 = jnp.bfloat16
f32 = jnp.float32


def _mm(a, b):
    return jnp.dot(a, b, preferred_element_type=f32)


def _mm_nt(a, b):
    return jax.lax.dot_general(a, b, NT, preferred_element_type=f32)


def _cat(ref, lo, hi):
    return jnp.concatenate([ref[u, lo:hi, :] for u in range(ref.shape[0])], axis=1)


def _ln(x):
    m = jnp.mean(x, axis=-1, keepdims=True)
    xc = x - m
    v = jnp.mean(xc * xc, axis=-1, keepdims=True)
    return xc * jax.lax.rsqrt(v + EPS)


def _gelu(x):
    k0 = math.sqrt(2.0 / math.pi)
    return 0.5 * x * (1.0 + jnp.tanh(k0 * (x + 0.044715 * (x * x * x))))


def _kernel(c_ref, x_hbm, ckv_hbm, wq_hbm, wuk_hbm, wuv_hbm, wo_hbm,
            w1_hbm, w2_hbm, w3_hbm, w4_hbm, wmod_hbm,
            out_hbm,
            x_v, ckv_v, wq_raw0, wuk_raw0, wuv_raw0, wq_raw, wuk_raw, wuv_raw, wo_v,
            w1_v, w2_v, w3_v, w4_v, wmod_v,
            wq_t, wuk_t, wuv_t,
            mod_s, h_s, q_s, k_s, v_s, ctx_s, acc_s, hb_s, g_s, out_v, sems, wsems):
    def cp(i, src, dst):
        return pltpu.make_async_copy(src, dst, sems.at[i])

    XC = 4
    XR = S // XC
    cp_wmoda = [cp(t, wmod_hbm.at[t * (M // 2):(t + 1) * (M // 2), 0:2 * M],
                   wmod_v.at[t * (M // 2):(t + 1) * (M // 2), 0:2 * M]) for t in range(2)]
    cp_x = [cp(2 + t, x_hbm.at[t * XR:(t + 1) * XR, :], x_v.at[t * XR:(t + 1) * XR, :])
            for t in range(XC)]
    cp_ckv = [cp(6 + t, ckv_hbm.at[t * (S // 2):(t + 1) * (S // 2), :],
                 ckv_v.at[t * (S // 2):(t + 1) * (S // 2), :]) for t in range(2)]
    cp_wuk0 = cp(8, wuk_hbm.at[:, 0:HG, :], wuk_raw0)
    cp_wuv0 = cp(9, wuv_hbm.at[:, 0:HG, :], wuv_raw0)
    cp_wq0 = cp(10, wq_hbm.at[:, 0:HG, :], wq_raw0)
    cp_wmodb = cp(11, wmod_hbm.at[:, 2 * M:6 * M], wmod_v.at[:, 2 * M:6 * M])
    cp_w1 = cp(12, w1_hbm, w1_v)
    cp_w2 = cp(13, w2_hbm, w2_v)
    cp_w3 = cp(14, w3_hbm, w3_v)
    cp_w4 = cp(15, w4_hbm, w4_v)

    MQ, MK = M // PPG, DC // PPG

    def raw_copies(g):
        slot = g % 2
        h0 = pl.multiple_of((g // PPG + 1) * HG, HG)
        cidx = g % PPG
        return [
            pltpu.make_async_copy(src.at[pl.ds(cidx * mc, mc), pl.ds(h0, HG), :],
                                  raw.at[slot], wsems.at[slot, n])
            for n, (src, raw, mc) in enumerate(((wq_hbm, wq_raw, MQ), (wuk_hbm, wuk_raw, MK),
                                                (wuv_hbm, wuv_raw, MK)))]

    def wo_copy(g):
        return pltpu.make_async_copy(wo_hbm.at[g], wo_v.at[g], wsems.at[g % 2, 3])

    for c_ in [cp_wuk0] + cp_ckv + [cp_wuv0]:
        c_.start()
    g_s[0:PAD, :] = jnp.zeros((PAD, M), f32)
    g_s[PAD + S:PAD + S + PAD, :] = jnp.zeros((PAD, M), f32)
    cv = jnp.broadcast_to(c_ref[...].astype(f32), (16, M))
    sil = (cv * jax.nn.sigmoid(cv)).astype(bf16)

    def relayout0(raw, dst):
        t = jnp.swapaxes(raw[...], 0, 1)
        for j in range(HG):
            dst[j] = t[j]

    cp_wuk0.wait()
    for c_ in cp_wmoda:
        c_.start()
    relayout0(wuk_raw0, wuk_t)
    for c_ in cp_ckv:
        c_.wait()
    cp_x[XC - 1].start()
    cp_wq0.start()
    for r in range(NB):
        lo, hi = r * BQ, (r + 1) * BQ
        k_s[lo:hi, :] = _mm(ckv_v[lo:hi, :], wuk_t[0]).astype(bf16)
    cp_wuv0.wait()
    wo_copy(0).start()
    cp_x[XC - 2].start()
    relayout0(wuv_raw0, wuv_t)
    for r in range(NB):
        lo, hi = r * BQ, (r + 1) * BQ
        v_s[lo:hi, :] = _mm(ckv_v[lo:hi, :], wuv_t[0]).astype(bf16)

    for c_ in cp_wmoda:
        c_.wait()
    for c_ in raw_copies(0) + cp_x[:XC - 2][::-1]:
        c_.start()
    mod_s[:, 0:2 * M] = _mm(sil, wmod_v[:, 0:2 * M])[0:8, :]

    def mod(i):
        return mod_s[0:1, i * M:(i + 1) * M]

    def norm_x(t):
        sa, ca = mod(0) * QSCALE, (1.0 + mod(1)) * QSCALE
        cp_x[t].wait()
        for r0 in range(t * XR, (t + 1) * XR, BQ):
            xr = x_v[r0:r0 + BQ, :].astype(f32)
            hr = (_ln(xr) * ca + sa).astype(bf16)
            for u in range(M // D):
                h_s[u, r0:r0 + BQ, :] = hr[:, u * D:(u + 1) * D]

    norm_x(XC - 1)
    cp_wq0.wait()
    relayout0(wq_raw0, wq_t)


    NRAW = NP - PPG

    def head(g, first):
        if not first:
            wo_copy(g).wait()
        def when(cond, fn):
            if first:
                if cond:
                    fn()
            else:
                pl.when(cond)(fn)

        def raw_wait():
            for c_ in raw_copies(g):
                c_.wait()

        def raw_start():
            for c_ in raw_copies(g + 1):
                c_.start()

        if not first:
            when(g < NRAW, raw_wait)
            when(g + 1 < NRAW, raw_start)
            when(g + 1 < NP, wo_copy(g + 1).start)
        for gi, c_ in enumerate((cp_wmodb, cp_w1, cp_w2, cp_w3, cp_w4)):
            when(g == gi + 1, c_.start)

        st = {}

        def pq(i):
            lo, hi = i * BQ, (i + 1) * BQ
            q_s[lo:hi, :] = _mm(_cat(h_s, lo, hi), wq_t[g]).astype(bf16)

        def pk(i):
            lo, hi = i * BQ, (i + 1) * BQ
            k_s[lo:hi, :] = _mm(ckv_v[lo:hi, :], wuk_t[g]).astype(bf16)

        def pv(i):
            lo, hi = i * BQ, (i + 1) * BQ
            v_s[lo:hi, :] = _mm(ckv_v[lo:hi, :], wuv_t[g]).astype(bf16)

        def po(i, gg):
            lo, hi = i * BQ, (i + 1) * BQ
            if first:
                acc_s[lo:hi, :] = _mm(ctx_s[lo:hi, :], wo_v[gg])
            else:
                acc_s[lo:hi, :] += _mm(ctx_s[lo:hi, :], wo_v[gg])

        def nkc(i):
            return i * BQ // KC

        def qk_chunk(i, j, c):
            lo = i * BQ
            cl, ch = j * D, (j + 1) * D
            d = st.setdefault((i, j), dict(s=[], mx=None))
            if c == 0:
                d['q'] = q_s[lo:lo + BQ, cl:ch]
            q = d['q']
            if c < nkc(i):
                sc = _mm_nt(q, k_s[c * KC:(c + 1) * KC, cl:ch])
                d['s'].append(sc)
                t = functools.reduce(jnp.maximum, [sc[:, u:u + D] for u in range(0, KC, D)])
                d['mx'] = t if d['mx'] is None else jnp.maximum(d['mx'], t)
            else:
                r = jax.lax.broadcasted_iota(jnp.int32, (D, D), 0)
                cc = jax.lax.broadcasted_iota(jnp.int32, (D, D), 1)
                tri = cc <= r
                mx = d['mx']
                tiles = []
                for t in range(BQ // D):
                    st_ = _mm_nt(q[t * D:], k_s[lo + t * D:lo + (t + 1) * D, cl:ch])
                    top = jnp.where(tri, st_[:D], NEG)
                    st_ = top if t == BQ // D - 1 else jnp.concatenate([top, st_[D:]], axis=0)
                    tiles.append(st_)
                    if mx is None:
                        mx = st_
                    elif t == 0:
                        mx = jnp.maximum(mx, st_)
                    else:
                        mx = jnp.concatenate([mx[:t * D], jnp.maximum(mx[t * D:], st_)], axis=0)
                d['s'].append(tiles)
                d['m'] = jnp.max(mx, axis=1, keepdims=True)

        def epv_chunk(i, j, c):
            lo = i * BQ
            cl, ch = j * D, (j + 1) * D
            d = st[(i, j)]
            m = d['m']
            if c < nkc(i):
                sc = d['s'][c]
                ps = [jnp.exp2(sc[:, u:u + D] - m) for u in range(0, KC, D)]
                pb = jnp.concatenate([p_.astype(bf16) for p_ in ps], axis=1)
                o = _mm(pb, v_s[c * KC:(c + 1) * KC, cl:ch])
                d['acc'] = o if c == 0 else d['acc'] + o
                t = functools.reduce(jnp.add, ps)
                d['l'] = t if c == 0 else d['l'] + t
            else:
                l = d['l'] if c > 0 else None
                acc = d['acc'] if c > 0 else None
                for t, st_ in enumerate(d['s'][c]):
                    p = jnp.exp2(st_ - m[t * D:])
                    o = _mm(p.astype(bf16), v_s[lo + t * D:lo + (t + 1) * D, cl:ch])
                    if l is None:
                        l, acc = p, o
                    elif t == 0:
                        l, acc = l + p, acc + o
                    else:
                        l = jnp.concatenate([l[:t * D], l[t * D:] + p], axis=0)
                        acc = jnp.concatenate([acc[:t * D], acc[t * D:] + o], axis=0)
                lsum = jnp.sum(l, axis=1, keepdims=True)
                ctx_s[lo:lo + BQ, cl:ch] = (acc / lsum).astype(bf16)

        def phase(qk_unit, epv_unit, fillers):
            nq = nkc(qk_unit[0]) + 1 if qk_unit is not None else 0
            ne = nkc(epv_unit[0]) + 1 if epv_unit is not None else 0
            n = max(nq, ne)
            nf = len(fillers)
            fpos = [((2 * t + 1) * n) // (2 * nf) for t in range(nf)]
            for c in range(n):
                if c < nq:
                    qk_chunk(qk_unit[0], qk_unit[1], c)
                for t in range(nf):
                    if fpos[t] == c:
                        fillers[t]()
                if c < ne:
                    epv_chunk(epv_unit[0], epv_unit[1], c)

        def relayout():
            slot = g % 2
            cidx = g % PPG
            for raw, dst, mc in ((wq_raw, wq_t, MQ), (wuk_raw, wuk_t, MK), (wuv_raw, wuv_t, MK)):
                t = jnp.swapaxes(raw[slot], 0, 1)
                r0 = pl.multiple_of(cidx * mc, 16)
                for j in range(HG):
                    pidx = ((g // PPG + 1) * PPG + j) % NP
                    dst[pidx, pl.ds(r0, mc), :] = t[j]

        P = functools.partial
        pq(NB - 1)
        if not first:
            for c in range(LAG):
                pk(c)
            po(ORDER[-1], g - 1)
        pq(NB - 2)
        R = BQ // KC
        for c in range(NB):
            if c + LAG < NB and not first:
                pk(c + LAG)
            for cc_ in range(c * R, (c + 1) * R if c < NB - 1 else c * R + 1):
                qk_chunk(NB - 1, 0, cc_)
            if not first:
                pv(c)
        for n, i in enumerate(ORDER):
            if first:
                if n == 0:
                    wo_copy(0).wait()
                if n + 2 < NB and n % 2 == 0:
                    norm_x(XC - 2 - n // 2)
                if n == 2:
                    raw_start()
                    wo_copy(1).start()
                if n == TPOS:
                    raw_wait()
            f = []
            if n + 2 < NB:
                f += [P(pq, ORDER[n + 2])]
            if n >= 1:
                f += [P(po, ORDER[n - 1], g)]
            if n == TPOS:
                f += [relayout]
            phase((ORDER[n + 1], 0) if n + 1 < NB else None, (i, 0), f)

    head(0, True)
    acc_s[ORDER[-1] * BQ:(ORDER[-1] + 1) * BQ, :] = jnp.zeros((BQ, M), f32)

    def body(g, carry):
        head(g, False)
        return carry

    jax.lax.fori_loop(1, NP, body, 0)
    lo_, hi_ = ORDER[-1] * BQ, (ORDER[-1] + 1) * BQ
    acc_s[lo_:hi_, :] += _mm(ctx_s[lo_:hi_, :], wo_v[NP - 1])

    cp_wmodb.wait()
    mod_s[:, 2 * M:6 * M] = _mm(sil, wmod_v[:, 2 * M:6 * M])[0:8, :]
    ga, sb, cb, gb = mod(2), mod(3), mod(4), mod(5)
    cp_w1.wait()
    cp_w2.wait()
    cp_w3.wait()
    cp_w4.wait()
    NR = S // BM
    lane = jax.lax.broadcasted_iota(jnp.int32, (BM, 128), 1)
    cp_out = [cp(16 + r, out_v.at[r * BM:(r + 1) * BM, :], out_hbm.at[0, r * BM:(r + 1) * BM, :])
              for r in range(NR)]
    fchunks = [(lo, min(lo + FC, F)) for lo in range(0, F, FC)]
    sv = {}

    def stage1(r):
        lo, hi = r * BM, (r + 1) * BM
        x1 = x_v[lo:hi, :].astype(f32) + ga * acc_s[lo:hi, :]
        hb = _ln(x1) * (1.0 + cb) + sb
        acc_s[lo:hi, :] = x1
        hb_s[lo:hi, :] = hb
        u = _ln(hb).astype(bf16)
        g_s[PAD + lo:PAD + hi, :] = _gelu(_mm(u, w1_v[...]))

    def mix(r):
        lo, hi = r * BM, (r + 1) * BM

        def sh(d, t):
            return g_s[PAD + lo + d:PAD + hi + d, t * 128:(t + 1) * 128]

        t0 = sh(-1, 0)
        t1 = jnp.where(lane < 32, sh(-1, 1), sh(1, 1))
        t2 = jnp.where(lane < 64, sh(1, 2), sh(-2, 2))
        t3 = jnp.where(lane < 96, sh(-2, 3), sh(2, 3))
        t4 = sh(2, 4)
        gs = jnp.concatenate([t0, t1, t2, t3, t4], axis=1).astype(bf16)
        sv[r] = dict(xb=hb_s[lo:hi, :] + _mm(gs, w2_v[...]))

    def norm(r):
        sv[r]['u'] = _ln(sv[r]['xb']).astype(bf16)

    def up(r, c):
        lo, hi = fchunks[c]
        sv[r][('h', c)] = _mm_nt(sv[r]['u'], w3_v[lo:hi, :])

    def down(r, c):
        lo, hi = fchunks[c]
        o = _mm(_gelu(sv[r][('h', c)]).astype(bf16), w4_v[lo:hi, :])
        sv[r]['o'] = o if c == 0 else sv[r]['o'] + o

    def finish(r):
        lo, hi = r * BM, (r + 1) * BM
        out_v[lo:hi, :] = (acc_s[lo:hi, :] + gb * (sv[r]['xb'] + sv[r]['o'])).astype(bf16)
        cp_out[r].start()

    nc = len(fchunks)
    for r in range(3):
        stage1(r)
    for r in range(2):
        mix(r)
    for r in range(2):
        norm(r)
    for r in range(NR):
        up(r, 0)
        for c in range(nc):
            if c + 1 < nc:
                up(r, c + 1)
            if c == 0 and 3 <= r + 2 < NR:
                stage1(r + 2)
            if c == 2 and 2 <= r + 1 < NR:
                mix(r + 1)
            if c == 3 and 2 <= r + 1 < NR:
                norm(r + 1)
            down(r, c)
        finish(r)
    for r in range(NR):
        cp_out[r].wait()


@jax.jit
def pallas_adaLN_cond__compressed_kv_cla__mixer_s_mlp__prompt_kernel(
    A_x: jax.Array,
    A_c_kv: jax.Array,
    A_w_q: jax.Array,
    A_w_uk: jax.Array,
    A_w_uv: jax.Array,
    A_w_o: jax.Array,
    B_x: jax.Array,
    B_w1: jax.Array,
    B_w2: jax.Array,
    B_w3: jax.Array,
    B_w4: jax.Array,
    c: jax.Array,
    w_mod: jax.Array,
):
    del B_x
    any_spec = pl.BlockSpec(memory_space=pltpu.HBM)
    V = pltpu.VMEM
    scratch = [
        V((S, M), bf16), V((S, DC), bf16),
        V((M, HG, D), bf16), V((DC, HG, D), bf16), V((DC, HG, D), bf16),
        V((2, M // PPG, HG, D), bf16), V((2, DC // PPG, HG, D), bf16), V((2, DC // PPG, HG, D), bf16),
        V((NP, HC * D, M), bf16),
        V((M, M), bf16), V((M, M), bf16), V((F, M), bf16), V((F, M), bf16), V((M, 6 * M), bf16),
        V((NP, M, HC * D), bf16), V((NP, DC, HC * D), bf16), V((NP, DC, HC * D), bf16),
        V((8, 6 * M), f32), V((M // D, S, D), bf16),
        V((S, HC * D), bf16), V((S, HC * D), bf16), V((S, HC * D), bf16), V((S, HC * D), bf16),
        V((S, M), f32), V((S, M), f32), V((S + 2 * PAD, M), f32), V((S, M), bf16),
        pltpu.SemaphoreType.DMA((16 + S // BM,)),
        pltpu.SemaphoreType.DMA((2, 4)),
    ]
    out = pl.pallas_call(
        _kernel,
        out_shape=jax.ShapeDtypeStruct((1, S, M), bf16),
        in_specs=[pl.BlockSpec(memory_space=pltpu.VMEM)] + [any_spec] * 11,
        out_specs=any_spec,
        scratch_shapes=scratch,
        compiler_params=pltpu.CompilerParams(vmem_limit_bytes=120 * 1024 * 1024),
    )(c, A_x.reshape(S, M), A_c_kv.reshape(S, DC), A_w_q, A_w_uk, A_w_uv, A_w_o.reshape(NP, HC * D, M),
      B_w1, B_w2, B_w3.T, B_w4, w_mod)
    return out
```

```python
import functools
import math

import jax
import jax.numpy as jnp
import jax.experimental.pallas as pl
import jax.experimental.pallas.tpu as pltpu

S = 2048
M = 640
H = 32
D = 128
DC = 4 * D
F = 1728
HG = 8
NG = H // HG
HC = 1
NP = H // HC
PPG = HG // HC
BQ = 256
NB = S // BQ
KC = 256
ORDER = (7, 6, 5, 4, 3, 2, 0, 1)
TPOS = 7
LAG = 3
BM = 128
FC = 512
PAD = 8
EPS = 1e-05
LOG2E = math.log2(math.e)
NT = (((1,), (1,)), ((), ()))
NEG = -1000000000.0 * LOG2E
QSCALE = (D ** -0.5) * LOG2E
bf16 = jnp.bfloat16
f32 = jnp.float32


def _mm(a, b):
    return jnp.dot(a, b, preferred_element_type=f32)


def _mm_nt(a, b):
    return jax.lax.dot_general(a, b, NT, preferred_element_type=f32)


def _cat(ref, lo, hi):
    return jnp.concatenate([ref[u, lo:hi, :] for u in range(ref.shape[0])], axis=1)


def _ln(x):
    m = jnp.mean(x, axis=-1, keepdims=True)
    xc = x - m
    v = jnp.mean(xc * xc, axis=-1, keepdims=True)
    return xc * jax.lax.rsqrt(v + EPS)


def _gelu(x):
    k0 = math.sqrt(2.0 / math.pi)
    return 0.5 * x * (1.0 + jnp.tanh(k0 * (x + 0.044715 * (x * x * x))))


def _kernel(c_ref, x_hbm, ckv_hbm, wq_hbm, wuk_hbm, wuv_hbm, wo_hbm,
            w1_hbm, w2_hbm, w3_hbm, w4_hbm, wmod_hbm,
            out_hbm,
            x_v, ckv_v, wq_raw0, wuk_raw0, wuv_raw0, wq_raw, wuk_raw, wuv_raw, wo_v,
            w1_v, w2_v, w3_v, w4_v, wmod_v,
            wq_t, wuk_t, wuv_t,
            mod_s, h_s, q_s, k_s, v_s, ctx_s, acc_s, hb_s, g_s, out_v, sems, wsems):
    def cp(i, src, dst):
        return pltpu.make_async_copy(src, dst, sems.at[i])

    XC = 4
    XR = S // XC
    cp_wmoda = [cp(t, wmod_hbm.at[t * (M // 2):(t + 1) * (M // 2), 0:2 * M],
                   wmod_v.at[t * (M // 2):(t + 1) * (M // 2), 0:2 * M]) for t in range(2)]
    cp_x = [cp(2 + t, x_hbm.at[t * XR:(t + 1) * XR, :], x_v.at[t * XR:(t + 1) * XR, :])
            for t in range(XC)]
    cp_ckv = [cp(6 + t, ckv_hbm.at[t * (S // 2):(t + 1) * (S // 2), :],
                 ckv_v.at[t * (S // 2):(t + 1) * (S // 2), :]) for t in range(2)]
    cp_wuk0 = cp(8, wuk_hbm.at[:, 0:HG, :], wuk_raw0)
    cp_wuv0 = cp(9, wuv_hbm.at[:, 0:HG, :], wuv_raw0)
    cp_wq0 = cp(10, wq_hbm.at[:, 0:HG, :], wq_raw0)
    cp_wmodb = cp(11, wmod_hbm.at[:, 2 * M:6 * M], wmod_v.at[:, 2 * M:6 * M])
    cp_w1 = cp(12, w1_hbm, w1_v)
    cp_w2 = cp(13, w2_hbm, w2_v)
    cp_w3 = cp(14, w3_hbm, w3_v)
    cp_w4 = cp(15, w4_hbm, w4_v)

    MQ, MK = M // PPG, DC // PPG

    def raw_copies(g):
        slot = g % 2
        h0 = pl.multiple_of((g // PPG + 1) * HG, HG)
        cidx = g % PPG
        return [
            pltpu.make_async_copy(src.at[pl.ds(cidx * mc, mc), pl.ds(h0, HG), :],
                                  raw.at[slot], wsems.at[slot, n])
            for n, (src, raw, mc) in enumerate(((wq_hbm, wq_raw, MQ), (wuk_hbm, wuk_raw, MK),
                                                (wuv_hbm, wuv_raw, MK)))]

    def wo_copy(g):
        return pltpu.make_async_copy(wo_hbm.at[g], wo_v.at[g], wsems.at[g % 2, 3])

    for c_ in [cp_wuk0] + cp_ckv + [cp_wuv0]:
        c_.start()
    g_s[0:PAD, :] = jnp.zeros((PAD, M), f32)
    g_s[PAD + S:PAD + S + PAD, :] = jnp.zeros((PAD, M), f32)
    cv = jnp.broadcast_to(c_ref[...].astype(f32), (16, M))
    sil = (cv * jax.nn.sigmoid(cv)).astype(bf16)

    def relayout0(raw, dst):
        t = jnp.swapaxes(raw[...], 0, 1)
        for j in range(HG):
            dst[j] = t[j]

    cp_wuk0.wait()
    for c_ in cp_wmoda:
        c_.start()
    relayout0(wuk_raw0, wuk_t)
    for c_ in cp_ckv:
        c_.wait()
    cp_x[XC - 1].start()
    cp_wq0.start()
    for r in range(NB):
        lo, hi = r * BQ, (r + 1) * BQ
        k_s[lo:hi, :] = _mm(ckv_v[lo:hi, :], wuk_t[0]).astype(bf16)
    cp_wuv0.wait()
    wo_copy(0).start()
    cp_x[XC - 2].start()
    relayout0(wuv_raw0, wuv_t)
    for r in range(NB):
        lo, hi = r * BQ, (r + 1) * BQ
        v_s[lo:hi, :] = _mm(ckv_v[lo:hi, :], wuv_t[0]).astype(bf16)

    for c_ in cp_wmoda:
        c_.wait()
    for c_ in raw_copies(0) + cp_x[:XC - 2][::-1]:
        c_.start()
    mod_s[:, 0:2 * M] = _mm(sil, wmod_v[:, 0:2 * M])[0:8, :]

    def mod(i):
        return mod_s[0:1, i * M:(i + 1) * M]

    def norm_x(t):
        sa, ca = mod(0) * QSCALE, (1.0 + mod(1)) * QSCALE
        cp_x[t].wait()
        for r0 in range(t * XR, (t + 1) * XR, BQ):
            xr = x_v[r0:r0 + BQ, :].astype(f32)
            hr = (_ln(xr) * ca + sa).astype(bf16)
            for u in range(M // D):
                h_s[u, r0:r0 + BQ, :] = hr[:, u * D:(u + 1) * D]

    norm_x(XC - 1)
    cp_wq0.wait()
    relayout0(wq_raw0, wq_t)


    NRAW = NP - PPG

    def head(g, first):
        if not first:
            wo_copy(g).wait()
        def when(cond, fn):
            if first:
                if cond:
                    fn()
            else:
                pl.when(cond)(fn)

        def raw_wait():
            for c_ in raw_copies(g):
                c_.wait()

        def raw_start():
            for c_ in raw_copies(g + 1):
                c_.start()

        if not first:
            when(g < NRAW, raw_wait)
            when(g + 1 < NRAW, raw_start)
            when(g + 1 < NP, wo_copy(g + 1).start)
        for gi, c_ in enumerate((cp_wmodb, cp_w1, cp_w2, cp_w3, cp_w4)):
            when(g == gi + 1, c_.start)

        st = {}

        def pq(i):
            lo, hi = i * BQ, (i + 1) * BQ
            q_s[lo:hi, :] = _mm(_cat(h_s, lo, hi), wq_t[g]).astype(bf16)

        def pk(i):
            lo, hi = i * BQ, (i + 1) * BQ
            k_s[lo:hi, :] = _mm(ckv_v[lo:hi, :], wuk_t[g]).astype(bf16)

        def pv(i):
            lo, hi = i * BQ, (i + 1) * BQ
            v_s[lo:hi, :] = _mm(ckv_v[lo:hi, :], wuv_t[g]).astype(bf16)

        def po(i, gg):
            lo, hi = i * BQ, (i + 1) * BQ
            if first:
                acc_s[lo:hi, :] = _mm(ctx_s[lo:hi, :], wo_v[gg])
            else:
                acc_s[lo:hi, :] += _mm(ctx_s[lo:hi, :], wo_v[gg])

        def nkc(i):
            return i * BQ // KC

        def qk_chunk(i, j, c):
            lo = i * BQ
            cl, ch = j * D, (j + 1) * D
            d = st.setdefault((i, j), dict(s=[], mx=None))
            if c == 0:
                d['q'] = q_s[lo:lo + BQ, cl:ch]
            q = d['q']
            if c < nkc(i):
                sc = _mm_nt(q, k_s[c * KC:(c + 1) * KC, cl:ch])
                d['s'].append(sc)
                t = functools.reduce(jnp.maximum, [sc[:, u:u + D] for u in range(0, KC, D)])
                d['mx'] = t if d['mx'] is None else jnp.maximum(d['mx'], t)
            else:
                r = jax.lax.broadcasted_iota(jnp.int32, (D, D), 0)
                cc = jax.lax.broadcasted_iota(jnp.int32, (D, D), 1)
                tri = cc <= r
                mx = d['mx']
                tiles = []
                for t in range(BQ // D):
                    st_ = _mm_nt(q[t * D:], k_s[lo + t * D:lo + (t + 1) * D, cl:ch])
                    top = jnp.where(tri, st_[:D], NEG)
                    st_ = top if t == BQ // D - 1 else jnp.concatenate([top, st_[D:]], axis=0)
                    tiles.append(st_)
                    if mx is None:
                        mx = st_
                    elif t == 0:
                        mx = jnp.maximum(mx, st_)
                    else:
                        mx = jnp.concatenate([mx[:t * D], jnp.maximum(mx[t * D:], st_)], axis=0)
                d['s'].append(tiles)
                d['m'] = jnp.max(mx, axis=1, keepdims=True)

        def epv_chunk(i, j, c):
            lo = i * BQ
            cl, ch = j * D, (j + 1) * D
            d = st[(i, j)]
            m = d['m']
            if c < nkc(i):
                sc = d['s'][c]
                ps = [jnp.exp2(sc[:, u:u + D] - m) for u in range(0, KC, D)]
                pb = jnp.concatenate([p_.astype(bf16) for p_ in ps], axis=1)
                o = _mm(pb, v_s[c * KC:(c + 1) * KC, cl:ch])
                d['acc'] = o if c == 0 else d['acc'] + o
                t = functools.reduce(jnp.add, ps)
                d['l'] = t if c == 0 else d['l'] + t
            else:
                l = d['l'] if c > 0 else None
                acc = d['acc'] if c > 0 else None
                for t, st_ in enumerate(d['s'][c]):
                    p = jnp.exp2(st_ - m[t * D:])
                    o = _mm(p.astype(bf16), v_s[lo + t * D:lo + (t + 1) * D, cl:ch])
                    if l is None:
                        l, acc = p, o
                    elif t == 0:
                        l, acc = l + p, acc + o
                    else:
                        l = jnp.concatenate([l[:t * D], l[t * D:] + p], axis=0)
                        acc = jnp.concatenate([acc[:t * D], acc[t * D:] + o], axis=0)
                lsum = jnp.sum(l, axis=1, keepdims=True)
                ctx_s[lo:lo + BQ, cl:ch] = (acc / lsum).astype(bf16)

        def phase(qk_unit, epv_unit, fillers):
            nq = nkc(qk_unit[0]) + 1 if qk_unit is not None else 0
            ne = nkc(epv_unit[0]) + 1 if epv_unit is not None else 0
            n = max(nq, ne)
            nf = len(fillers)
            fpos = [((2 * t + 1) * n) // (2 * nf) for t in range(nf)]
            for c in range(n):
                if c < nq:
                    qk_chunk(qk_unit[0], qk_unit[1], c)
                for t in range(nf):
                    if fpos[t] == c:
                        fillers[t]()
                if c < ne:
                    epv_chunk(epv_unit[0], epv_unit[1], c)

        def relayout():
            slot = g % 2
            cidx = g % PPG
            for raw, dst, mc in ((wq_raw, wq_t, MQ), (wuk_raw, wuk_t, MK), (wuv_raw, wuv_t, MK)):
                t = jnp.swapaxes(raw[slot], 0, 1)
                r0 = pl.multiple_of(cidx * mc, 16)
                for j in range(HG):
                    pidx = ((g // PPG + 1) * PPG + j) % NP
                    dst[pidx, pl.ds(r0, mc), :] = t[j]

        P = functools.partial
        pq(NB - 1)
        if not first:
            for c in range(LAG):
                pk(c)
            po(ORDER[-1], g - 1)
        pq(NB - 2)
        R = BQ // KC
        for c in range(NB):
            if c + LAG < NB and not first:
                pk(c + LAG)
            for cc_ in range(c * R, (c + 1) * R if c < NB - 1 else c * R + 1):
                qk_chunk(NB - 1, 0, cc_)
            if not first:
                pv(c)
        for n, i in enumerate(ORDER):
            if first:
                if n == 0:
                    wo_copy(0).wait()
                if n + 2 < NB and n % 2 == 0:
                    norm_x(XC - 2 - n // 2)
                if n == 2:
                    raw_start()
                    wo_copy(1).start()
                if n == TPOS:
                    raw_wait()
            f = []
            if n + 2 < NB:
                f += [P(pq, ORDER[n + 2])]
            if n >= 1:
                f += [P(po, ORDER[n - 1], g)]
            if n == TPOS:
                f += [relayout]
            phase((ORDER[n + 1], 0) if n + 1 < NB else None, (i, 0), f)

    head(0, True)
    acc_s[ORDER[-1] * BQ:(ORDER[-1] + 1) * BQ, :] = jnp.zeros((BQ, M), f32)

    def body(g, carry):
        head(g, False)
        return carry

    jax.lax.fori_loop(1, NP, body, 0)
    for c_ in (cp_wmodb, cp_w1, cp_w2, cp_w3, cp_w4):
        c_.wait()
    lo_, hi_ = ORDER[-1] * BQ, (ORDER[-1] + 1) * BQ
    acc_s[lo_:hi_, :] += _mm(ctx_s[lo_:hi_, :], wo_v[NP - 1])
    mod_s[:, 2 * M:6 * M] = _mm(sil, wmod_v[:, 2 * M:6 * M])[0:8, :]
    ga, sb, cb, gb = mod(2), mod(3), mod(4), mod(5)
    NR = S // BM
    lane = jax.lax.broadcasted_iota(jnp.int32, (BM, 128), 1)
    cp_out = [cp(16 + r, out_v.at[r * BM:(r + 1) * BM, :], out_hbm.at[0, r * BM:(r + 1) * BM, :])
              for r in range(NR)]
    fchunks = [(lo, min(lo + FC, F)) for lo in range(0, F, FC)]
    sv = {}

    def stage1(r):
        lo, hi = r * BM, (r + 1) * BM
        x1 = x_v[lo:hi, :].astype(f32) + ga * acc_s[lo:hi, :]
        hb = _ln(x1) * (1.0 + cb) + sb
        acc_s[lo:hi, :] = x1
        hb_s[lo:hi, :] = hb
        u = _ln(hb).astype(bf16)
        g_s[PAD + lo:PAD + hi, :] = _gelu(_mm(u, w1_v[...]))

    def mix(r):
        lo, hi = r * BM, (r + 1) * BM

        def sh(d, t):
            return g_s[PAD + lo + d:PAD + hi + d, t * 128:(t + 1) * 128]

        t0 = sh(-1, 0)
        t1 = jnp.where(lane < 32, sh(-1, 1), sh(1, 1))
        t2 = jnp.where(lane < 64, sh(1, 2), sh(-2, 2))
        t3 = jnp.where(lane < 96, sh(-2, 3), sh(2, 3))
        t4 = sh(2, 4)
        gs = jnp.concatenate([t0, t1, t2, t3, t4], axis=1).astype(bf16)
        sv[r] = dict(xb=hb_s[lo:hi, :] + _mm(gs, w2_v[...]))

    def norm(r):
        sv[r]['u'] = _ln(sv[r]['xb']).astype(bf16)

    def up(r, c):
        lo, hi = fchunks[c]
        sv[r][('h', c)] = _mm_nt(sv[r]['u'], w3_v[lo:hi, :])

    def down(r, c):
        lo, hi = fchunks[c]
        o = _mm(_gelu(sv[r][('h', c)]).astype(bf16), w4_v[lo:hi, :])
        sv[r]['o'] = o if c == 0 else sv[r]['o'] + o

    def finish(r):
        lo, hi = r * BM, (r + 1) * BM
        out_v[lo:hi, :] = (acc_s[lo:hi, :] + gb * (sv[r]['xb'] + sv[r]['o'])).astype(bf16)
        cp_out[r].start()

    nc = len(fchunks)
    for r in range(3):
        stage1(r)
    for r in range(2):
        mix(r)
    for r in range(2):
        norm(r)
    for r in range(NR):
        up(r, 0)
        for c in range(nc):
            if c + 1 < nc:
                up(r, c + 1)
            if c == 0 and 3 <= r + 2 < NR:
                stage1(r + 2)
            if c == 2 and 2 <= r + 1 < NR:
                mix(r + 1)
            if c == 3 and 2 <= r + 1 < NR:
                norm(r + 1)
            down(r, c)
        finish(r)
    for r in range(NR):
        cp_out[r].wait()


@jax.jit
def pallas_adaLN_cond__compressed_kv_cla__mixer_s_mlp__prompt_kernel(
    A_x: jax.Array,
    A_c_kv: jax.Array,
    A_w_q: jax.Array,
    A_w_uk: jax.Array,
    A_w_uv: jax.Array,
    A_w_o: jax.Array,
    B_x: jax.Array,
    B_w1: jax.Array,
    B_w2: jax.Array,
    B_w3: jax.Array,
    B_w4: jax.Array,
    c: jax.Array,
    w_mod: jax.Array,
):
    del B_x
    any_spec = pl.BlockSpec(memory_space=pltpu.HBM)
    V = pltpu.VMEM
    scratch = [
        V((S, M), bf16), V((S, DC), bf16),
        V((M, HG, D), bf16), V((DC, HG, D), bf16), V((DC, HG, D), bf16),
        V((2, M // PPG, HG, D), bf16), V((2, DC // PPG, HG, D), bf16), V((2, DC // PPG, HG, D), bf16),
        V((NP, HC * D, M), bf16),
        V((M, M), bf16), V((M, M), bf16), V((F, M), bf16), V((F, M), bf16), V((M, 6 * M), bf16),
        V((NP, M, HC * D), bf16), V((NP, DC, HC * D), bf16), V((NP, DC, HC * D), bf16),
        V((8, 6 * M), f32), V((M // D, S, D), bf16),
        V((S, HC * D), bf16), V((S, HC * D), bf16), V((S, HC * D), bf16), V((S, HC * D), bf16),
        V((S, M), f32), V((S, M), f32), V((S + 2 * PAD, M), f32), V((S, M), bf16),
        pltpu.SemaphoreType.DMA((16 + S // BM,)),
        pltpu.SemaphoreType.DMA((2, 4)),
    ]
    out = pl.pallas_call(
        _kernel,
        out_shape=jax.ShapeDtypeStruct((1, S, M), bf16),
        in_specs=[pl.BlockSpec(memory_space=pltpu.VMEM)] + [any_spec] * 11,
        out_specs=any_spec,
        scratch_shapes=scratch,
        compiler_params=pltpu.CompilerParams(
            vmem_limit_bytes=120 * 1024 * 1024,
            disable_bounds_checks=True,
        ),
    )(c, A_x.reshape(S, M), A_c_kv.reshape(S, DC), A_w_q, A_w_uk, A_w_uv, A_w_o.reshape(NP, HC * D, M),
      B_w1, B_w2, B_w3.T, B_w4, w_mod)
    return out
```

```python
import functools
import math

import jax
import jax.numpy as jnp
import jax.experimental.pallas as pl
import jax.experimental.pallas.tpu as pltpu

S = 2048
M = 640
H = 32
D = 128
DC = 4 * D
F = 1728
HG = 8
NP = H
PPG = HG
BQ = 256
NB = S // BQ
KC = 256
ORDER = (7, 6, 5, 4, 3, 2, 0, 1)
TPOS = 7
LAG = 3
BM = 128
FC = 512
PAD = 8
EPS = 1e-05
LOG2E = math.log2(math.e)
NT = (((1,), (1,)), ((), ()))
NEG = -1000000000.0 * LOG2E
QSCALE = (D ** -0.5) * LOG2E
bf16 = jnp.bfloat16
f32 = jnp.float32


def _mm(a, b):
    return jnp.dot(a, b, preferred_element_type=f32)


def _mm_nt(a, b):
    return jax.lax.dot_general(a, b, NT, preferred_element_type=f32)


def _cat(ref, lo, hi):
    return jnp.concatenate([ref[u, lo:hi, :] for u in range(ref.shape[0])], axis=1)


def _ln(x):
    m = jnp.mean(x, axis=-1, keepdims=True)
    xc = x - m
    v = jnp.mean(xc * xc, axis=-1, keepdims=True)
    return xc * jax.lax.rsqrt(v + EPS)


def _gelu(x):
    k0 = math.sqrt(2.0 / math.pi)
    return 0.5 * x * (1.0 + jnp.tanh(k0 * (x + 0.044715 * (x * x * x))))


def _kernel(c_ref, x_hbm, ckv_hbm, wq_hbm, wuk_hbm, wuv_hbm, wo_hbm,
            w1_hbm, w2_hbm, w3_hbm, w4_hbm, wmod_hbm,
            out_hbm,
            x_v, ckv_v, wq_raw0, wuk_raw0, wuv_raw0, wq_raw, wuk_raw, wuv_raw, wo_v,
            w1_v, w2_v, w3_v, w4_v, wmod_v,
            wq_t, wuk_t, wuv_t,
            mod_s, h_s, q_s, k_s, v_s, ctx_s, acc_s, hb_s, g_s, out_v, sems, wsems):
    def cp(i, src, dst):
        return pltpu.make_async_copy(src, dst, sems.at[i])

    XC = 4
    XR = S // XC
    cp_wmoda = [cp(t, wmod_hbm.at[t * (M // 2):(t + 1) * (M // 2), 0:2 * M],
                   wmod_v.at[t * (M // 2):(t + 1) * (M // 2), 0:2 * M]) for t in range(2)]
    cp_x = [cp(2 + t, x_hbm.at[t * XR:(t + 1) * XR, :], x_v.at[t * XR:(t + 1) * XR, :])
            for t in range(XC)]
    cp_ckv = [cp(6 + t, ckv_hbm.at[t * (S // 2):(t + 1) * (S // 2), :],
                 ckv_v.at[t * (S // 2):(t + 1) * (S // 2), :]) for t in range(2)]
    cp_wuk0 = cp(8, wuk_hbm.at[:, 0:HG, :], wuk_raw0)
    cp_wuv0 = cp(9, wuv_hbm.at[:, 0:HG, :], wuv_raw0)
    cp_wq0 = cp(10, wq_hbm.at[:, 0:HG, :], wq_raw0)
    cp_wmodb = cp(11, wmod_hbm.at[:, 2 * M:6 * M], wmod_v.at[:, 2 * M:6 * M])
    cp_w1 = cp(12, w1_hbm, w1_v)
    cp_w2 = cp(13, w2_hbm, w2_v)
    cp_w3 = cp(14, w3_hbm, w3_v)
    cp_w4 = cp(15, w4_hbm, w4_v)

    MQ, MK = M // PPG, DC // PPG

    def raw_copies(g):
        slot = g % 2
        h0 = pl.multiple_of((g // PPG + 1) * HG, HG)
        cidx = g % PPG
        return [
            pltpu.make_async_copy(src.at[pl.ds(cidx * mc, mc), pl.ds(h0, HG), :],
                                  raw.at[slot], wsems.at[slot, n])
            for n, (src, raw, mc) in enumerate(((wq_hbm, wq_raw, MQ), (wuk_hbm, wuk_raw, MK),
                                                (wuv_hbm, wuv_raw, MK)))]

    def wo_copy(g):
        return pltpu.make_async_copy(wo_hbm.at[g], wo_v.at[g], wsems.at[g % 2, 3])

    for c_ in [cp_wuk0] + cp_ckv + [cp_wuv0]:
        c_.start()
    g_s[0:PAD, :] = jnp.zeros((PAD, M), f32)
    g_s[PAD + S:PAD + S + PAD, :] = jnp.zeros((PAD, M), f32)
    cv = jnp.broadcast_to(c_ref[...].astype(f32), (16, M))
    sil = (cv * jax.nn.sigmoid(cv)).astype(bf16)

    def relayout0(raw, dst):
        t = jnp.swapaxes(raw[...], 0, 1)
        for j in range(HG):
            dst[j] = t[j]

    cp_wuk0.wait()
    for c_ in cp_wmoda:
        c_.start()
    relayout0(wuk_raw0, wuk_t)
    for c_ in cp_ckv:
        c_.wait()
    cp_x[XC - 1].start()
    cp_wq0.start()
    for r in range(NB):
        lo, hi = r * BQ, (r + 1) * BQ
        k_s[lo:hi, :] = _mm(ckv_v[lo:hi, :], wuk_t[0]).astype(bf16)
    cp_wuv0.wait()
    wo_copy(0).start()
    cp_x[XC - 2].start()
    relayout0(wuv_raw0, wuv_t)
    for r in range(NB):
        lo, hi = r * BQ, (r + 1) * BQ
        v_s[lo:hi, :] = _mm(ckv_v[lo:hi, :], wuv_t[0]).astype(bf16)

    for c_ in cp_wmoda:
        c_.wait()
    for c_ in raw_copies(0) + cp_x[:XC - 2][::-1]:
        c_.start()
    mod_s[:, 0:2 * M] = _mm(sil, wmod_v[:, 0:2 * M])[0:8, :]

    def mod(i):
        return mod_s[0:1, i * M:(i + 1) * M]

    def norm_x(t):
        sa, ca = mod(0) * QSCALE, (1.0 + mod(1)) * QSCALE
        cp_x[t].wait()
        for r0 in range(t * XR, (t + 1) * XR, BQ):
            xr = x_v[r0:r0 + BQ, :].astype(f32)
            hr = (_ln(xr) * ca + sa).astype(bf16)
            for u in range(M // D):
                h_s[u, r0:r0 + BQ, :] = hr[:, u * D:(u + 1) * D]

    norm_x(XC - 1)
    cp_wq0.wait()
    relayout0(wq_raw0, wq_t)

    NRAW = NP - PPG

    def head(g, first):
        if not first:
            wo_copy(g).wait()

        def when(cond, fn):
            if first:
                if cond:
                    fn()
            else:
                pl.when(cond)(fn)

        def raw_wait():
            for c_ in raw_copies(g):
                c_.wait()

        def raw_start():
            for c_ in raw_copies(g + 1):
                c_.start()

        if not first:
            when(g < NRAW, raw_wait)
            when(g + 1 < NRAW, raw_start)
            when(g + 1 < NP, wo_copy(g + 1).start)
        for gi, c_ in enumerate((cp_wmodb, cp_w1, cp_w2, cp_w3, cp_w4)):
            when(g == gi + 1, c_.start)

        st = {}

        def pq(i):
            lo, hi = i * BQ, (i + 1) * BQ
            q_s[lo:hi, :] = _mm(_cat(h_s, lo, hi), wq_t[g]).astype(bf16)

        def pk(i):
            lo, hi = i * BQ, (i + 1) * BQ
            k_s[lo:hi, :] = _mm(ckv_v[lo:hi, :], wuk_t[g]).astype(bf16)

        def pv(i):
            lo, hi = i * BQ, (i + 1) * BQ
            v_s[lo:hi, :] = _mm(ckv_v[lo:hi, :], wuv_t[g]).astype(bf16)

        def po(i, gg):
            lo, hi = i * BQ, (i + 1) * BQ
            if first:
                acc_s[lo:hi, :] = _mm(ctx_s[lo:hi, :], wo_v[gg])
            else:
                acc_s[lo:hi, :] += _mm(ctx_s[lo:hi, :], wo_v[gg])

        def nkc(i):
            return i * BQ // KC

        def qk_chunk(i, c):
            lo = i * BQ
            d = st.setdefault(i, dict(s=[], mx=None))
            if c == 0:
                d['q'] = q_s[lo:lo + BQ, :]
            q = d['q']
            if c < nkc(i):
                sc = _mm_nt(q, k_s[c * KC:(c + 1) * KC, :])
                d['s'].append(sc)
                t = functools.reduce(jnp.maximum, [sc[:, u:u + D] for u in range(0, KC, D)])
                d['mx'] = t if d['mx'] is None else jnp.maximum(d['mx'], t)
            else:
                r = jax.lax.broadcasted_iota(jnp.int32, (D, D), 0)
                cc = jax.lax.broadcasted_iota(jnp.int32, (D, D), 1)
                tri = cc <= r
                mx = d['mx']
                tiles = []
                for t in range(BQ // D):
                    st_ = _mm_nt(q[t * D:], k_s[lo + t * D:lo + (t + 1) * D, :])
                    top = jnp.where(tri, st_[:D], NEG)
                    st_ = top if t == BQ // D - 1 else jnp.concatenate([top, st_[D:]], axis=0)
                    tiles.append(st_)
                    if mx is None:
                        mx = st_
                    elif t == 0:
                        mx = jnp.maximum(mx, st_)
                    else:
                        mx = jnp.concatenate([mx[:t * D], jnp.maximum(mx[t * D:], st_)], axis=0)
                d['s'].append(tiles)
                d['m'] = jnp.max(mx, axis=1, keepdims=True)

        def epv_chunk(i, c):
            lo = i * BQ
            d = st[i]
            m = d['m']
            if c < nkc(i):
                sc = d['s'][c]
                ps = [jnp.exp2(sc[:, u:u + D] - m) for u in range(0, KC, D)]
                pb = jnp.concatenate([p_.astype(bf16) for p_ in ps], axis=1)
                o = _mm(pb, v_s[c * KC:(c + 1) * KC, :])
                d['acc'] = o if c == 0 else d['acc'] + o
                t = functools.reduce(jnp.add, ps)
                d['l'] = t if c == 0 else d['l'] + t
            else:
                l = d['l'] if c > 0 else None
                acc = d['acc'] if c > 0 else None
                for t, st_ in enumerate(d['s'][c]):
                    p = jnp.exp2(st_ - m[t * D:])
                    o = _mm(p.astype(bf16), v_s[lo + t * D:lo + (t + 1) * D, :])
                    if l is None:
                        l, acc = p, o
                    elif t == 0:
                        l, acc = l + p, acc + o
                    else:
                        l = jnp.concatenate([l[:t * D], l[t * D:] + p], axis=0)
                        acc = jnp.concatenate([acc[:t * D], acc[t * D:] + o], axis=0)
                lsum = jnp.sum(l, axis=1, keepdims=True)
                ctx_s[lo:lo + BQ, :] = (acc / lsum).astype(bf16)

        def phase(qk_unit, epv_unit, fillers):
            nq = nkc(qk_unit) + 1 if qk_unit is not None else 0
            ne = nkc(epv_unit) + 1 if epv_unit is not None else 0
            n = max(nq, ne)
            nf = len(fillers)
            fpos = [((2 * t + 1) * n) // (2 * nf) for t in range(nf)]
            for c in range(n):
                if c < nq:
                    qk_chunk(qk_unit, c)
                for t in range(nf):
                    if fpos[t] == c:
                        fillers[t]()
                if c < ne:
                    epv_chunk(epv_unit, c)

        def relayout():
            slot = g % 2
            cidx = g % PPG
            for raw, dst, mc in ((wq_raw, wq_t, MQ), (wuk_raw, wuk_t, MK), (wuv_raw, wuv_t, MK)):
                t = jnp.swapaxes(raw[slot], 0, 1)
                r0 = pl.multiple_of(cidx * mc, 16)
                for j in range(HG):
                    pidx = ((g // PPG + 1) * PPG + j) % NP
                    dst[pidx, pl.ds(r0, mc), :] = t[j]

        P = functools.partial
        pq(ORDER[0])
        if not first:
            for c in range(LAG):
                pk(c)
            po(ORDER[-1], g - 1)
        pq(ORDER[1])
        for c in range(NB):
            if c + LAG < NB and not first:
                pk(c + LAG)
            qk_chunk(ORDER[0], c)
            if not first:
                pv(c)
        for n, i in enumerate(ORDER):
            if first:
                if n == 0:
                    wo_copy(0).wait()
                if n + 2 < NB and n % 2 == 0:
                    norm_x(XC - 2 - n // 2)
                if n == 2:
                    raw_start()
                    wo_copy(1).start()
                if n == TPOS:
                    raw_wait()
            f = []
            if n + 2 < NB:
                f += [P(pq, ORDER[n + 2])]
            if n >= 1:
                f += [P(po, ORDER[n - 1], g)]
            if n == TPOS:
                f += [relayout]
            phase(ORDER[n + 1] if n + 1 < NB else None, i, f)

    head(0, True)
    acc_s[ORDER[-1] * BQ:(ORDER[-1] + 1) * BQ, :] = jnp.zeros((BQ, M), f32)

    def body(g, carry):
        head(g, False)
        return carry

    jax.lax.fori_loop(1, NP, body, 0)

    for c_ in (cp_wmodb, cp_w1, cp_w2, cp_w3, cp_w4):
        c_.wait()
    lo_, hi_ = ORDER[-1] * BQ, (ORDER[-1] + 1) * BQ
    acc_s[lo_:hi_, :] += _mm(ctx_s[lo_:hi_, :], wo_v[NP - 1])
    mod_s[:, 2 * M:6 * M] = _mm(sil, wmod_v[:, 2 * M:6 * M])[0:8, :]
    ga, sb, cb, gb = mod(2), mod(3), mod(4), mod(5)
    NR = S // BM
    lane = jax.lax.broadcasted_iota(jnp.int32, (BM, 128), 1)
    cp_out = [cp(16 + r, out_v.at[r * BM:(r + 1) * BM, :], out_hbm.at[0, r * BM:(r + 1) * BM, :])
              for r in range(NR)]
    fchunks = [(lo, min(lo + FC, F)) for lo in range(0, F, FC)]
    sv = {}

    def stage1(r):
        lo, hi = r * BM, (r + 1) * BM
        x1 = x_v[lo:hi, :].astype(f32) + ga * acc_s[lo:hi, :]
        hb = _ln(x1) * (1.0 + cb) + sb
        acc_s[lo:hi, :] = x1
        hb_s[lo:hi, :] = hb
        u = _ln(hb).astype(bf16)
        g_s[PAD + lo:PAD + hi, :] = _gelu(_mm(u, w1_v[...]))

    def mix(r):
        lo, hi = r * BM, (r + 1) * BM

        def sh(d, t):
            return g_s[PAD + lo + d:PAD + hi + d, t * 128:(t + 1) * 128]

        t0 = sh(-1, 0)
        t1 = jnp.where(lane < 32, sh(-1, 1), sh(1, 1))
        t2 = jnp.where(lane < 64, sh(1, 2), sh(-2, 2))
        t3 = jnp.where(lane < 96, sh(-2, 3), sh(2, 3))
        t4 = sh(2, 4)
        gs = jnp.concatenate([t0, t1, t2, t3, t4], axis=1).astype(bf16)
        sv[r] = dict(xb=hb_s[lo:hi, :] + _mm(gs, w2_v[...]))

    def norm(r):
        sv[r]['u'] = _ln(sv[r]['xb']).astype(bf16)

    def up(r, c):
        lo, hi = fchunks[c]
        sv[r][('h', c)] = _mm_nt(sv[r]['u'], w3_v[lo:hi, :])

    def down(r, c):
        lo, hi = fchunks[c]
        o = _mm(_gelu(sv[r][('h', c)]).astype(bf16), w4_v[lo:hi, :])
        sv[r]['o'] = o if c == 0 else sv[r]['o'] + o

    def finish(r):
        lo, hi = r * BM, (r + 1) * BM
        out_v[lo:hi, :] = (acc_s[lo:hi, :] + gb * (sv[r]['xb'] + sv[r]['o'])).astype(bf16)
        cp_out[r].start()

    nc = len(fchunks)
    for r in range(3):
        stage1(r)
    for r in range(2):
        mix(r)
    for r in range(2):
        norm(r)
    for r in range(NR):
        up(r, 0)
        for c in range(nc):
            if c + 1 < nc:
                up(r, c + 1)
            if c == 0 and 3 <= r + 2 < NR:
                stage1(r + 2)
            if c == 2 and 2 <= r + 1 < NR:
                mix(r + 1)
            if c == 3 and 2 <= r + 1 < NR:
                norm(r + 1)
            down(r, c)
        finish(r)
    for r in range(NR):
        cp_out[r].wait()


@jax.jit
def pallas_adaLN_cond__compressed_kv_cla__mixer_s_mlp__prompt_kernel(
    A_x: jax.Array,
    A_c_kv: jax.Array,
    A_w_q: jax.Array,
    A_w_uk: jax.Array,
    A_w_uv: jax.Array,
    A_w_o: jax.Array,
    B_x: jax.Array,
    B_w1: jax.Array,
    B_w2: jax.Array,
    B_w3: jax.Array,
    B_w4: jax.Array,
    c: jax.Array,
    w_mod: jax.Array,
):
    del B_x
    any_spec = pl.BlockSpec(memory_space=pltpu.HBM)
    V = pltpu.VMEM
    scratch = [
        V((S, M), bf16), V((S, DC), bf16),
        V((M, HG, D), bf16), V((DC, HG, D), bf16), V((DC, HG, D), bf16),
        V((2, M // PPG, HG, D), bf16), V((2, DC // PPG, HG, D), bf16), V((2, DC // PPG, HG, D), bf16),
        V((NP, D, M), bf16),
        V((M, M), bf16), V((M, M), bf16), V((F, M), bf16), V((F, M), bf16), V((M, 6 * M), bf16),
        V((NP, M, D), bf16), V((NP, DC, D), bf16), V((NP, DC, D), bf16),
        V((8, 6 * M), f32), V((M // D, S, D), bf16),
        V((S, D), bf16), V((S, D), bf16), V((S, D), bf16), V((S, D), bf16),
        V((S, M), f32), V((S, M), f32), V((S + 2 * PAD, M), f32), V((S, M), bf16),
        pltpu.SemaphoreType.DMA((16 + S // BM,)),
        pltpu.SemaphoreType.DMA((2, 4)),
    ]
    out = pl.pallas_call(
        _kernel,
        out_shape=jax.ShapeDtypeStruct((1, S, M), bf16),
        in_specs=[pl.BlockSpec(memory_space=pltpu.VMEM)] + [any_spec] * 11,
        out_specs=any_spec,
        scratch_shapes=scratch,
        compiler_params=pltpu.CompilerParams(
            vmem_limit_bytes=120 * 1024 * 1024,
            disable_bounds_checks=True,
        ),
    )(c, A_x.reshape(S, M), A_c_kv.reshape(S, DC), A_w_q, A_w_uk, A_w_uv, A_w_o.reshape(NP, D, M),
      B_w1, B_w2, B_w3.T, B_w4, w_mod)
    return out
```

```python
import functools
import math

import jax
import jax.numpy as jnp
import jax.experimental.pallas as pl
import jax.experimental.pallas.tpu as pltpu

S = 2048
M = 640
H = 32
D = 128
DC = 4 * D
F = 1728
HG = 8
NP = H
PPG = HG
BQ = 256
NB = S // BQ
KC = 256
ORDER = (7, 6, 5, 4, 3, 2, 0, 1)
TPOS = 7
LAG = 3
BM = 128
FC = 512
PAD = 8
EPS = 1e-05
LOG2E = math.log2(math.e)
NT = (((1,), (1,)), ((), ()))
NEG = -1000000000.0 * LOG2E
QSCALE = (D ** -0.5) * LOG2E
bf16 = jnp.bfloat16
f32 = jnp.float32


def _mm(a, b):
    return jnp.dot(a, b, preferred_element_type=f32)


def _mm_nt(a, b):
    return jax.lax.dot_general(a, b, NT, preferred_element_type=f32)


def _cat(ref, lo, hi):
    return jnp.concatenate([ref[u, lo:hi, :] for u in range(ref.shape[0])], axis=1)


def _ln(x):
    m = jnp.mean(x, axis=-1, keepdims=True)
    xc = x - m
    v = jnp.mean(xc * xc, axis=-1, keepdims=True)
    return xc * jax.lax.rsqrt(v + EPS)


def _gelu(x):
    k0 = math.sqrt(2.0 / math.pi)
    return 0.5 * x * (1.0 + jnp.tanh(k0 * (x + 0.044715 * (x * x * x))))


def _kernel(c_ref, x_hbm, ckv_hbm, wq_hbm, wuk_hbm, wuv_hbm, wo_hbm,
            w1_hbm, w2_hbm, w3_hbm, w4_hbm, wmod_hbm,
            out_hbm,
            x_v, ckv_v, wq_raw0, wuk_raw0, wuv_raw0, wq_raw, wuk_raw, wuv_raw, wo_v,
            w1_v, w2_v, w3_v, w4_v, wmod_v,
            wq_t, wuk_t, wuv_t,
            mod_s, h_s, q_s, k_s, v_s, ctx_s, acc_s, hb_s, g_s, out_v, sems, wsems):
    def cp(i, src, dst):
        return pltpu.make_async_copy(src, dst, sems.at[i])

    XC = 4
    XR = S // XC
    cp_wmoda = [cp(t, wmod_hbm.at[t * (M // 2):(t + 1) * (M // 2), 0:2 * M],
                   wmod_v.at[t * (M // 2):(t + 1) * (M // 2), 0:2 * M]) for t in range(2)]
    cp_x = [cp(2 + t, x_hbm.at[t * XR:(t + 1) * XR, :], x_v.at[t * XR:(t + 1) * XR, :])
            for t in range(XC)]
    cp_ckv = [cp(6 + t, ckv_hbm.at[t * (S // 2):(t + 1) * (S // 2), :],
                 ckv_v.at[t * (S // 2):(t + 1) * (S // 2), :]) for t in range(2)]
    cp_wuk0 = cp(8, wuk_hbm.at[:, 0:HG, :], wuk_raw0)
    cp_wuv0 = cp(9, wuv_hbm.at[:, 0:HG, :], wuv_raw0)
    cp_wq0 = cp(10, wq_hbm.at[:, 0:HG, :], wq_raw0)
    cp_wmodb = cp(11, wmod_hbm.at[:, 2 * M:6 * M], wmod_v.at[:, 2 * M:6 * M])
    cp_w1 = cp(12, w1_hbm, w1_v)
    cp_w2 = cp(13, w2_hbm, w2_v)
    cp_w3 = cp(14, w3_hbm, w3_v)
    cp_w4 = cp(15, w4_hbm, w4_v)

    MQ, MK = M // PPG, DC // PPG

    def raw_copies(g):
        slot = g % 2
        h0 = pl.multiple_of((g // PPG + 1) * HG, HG)
        cidx = g % PPG
        return [
            pltpu.make_async_copy(src.at[pl.ds(cidx * mc, mc), pl.ds(h0, HG), :],
                                  raw.at[slot], wsems.at[slot, n])
            for n, (src, raw, mc) in enumerate(((wq_hbm, wq_raw, MQ), (wuk_hbm, wuk_raw, MK),
                                                (wuv_hbm, wuv_raw, MK)))]

    def wo_copy(g):
        return pltpu.make_async_copy(wo_hbm.at[g], wo_v.at[g], wsems.at[g % 2, 3])

    for c_ in [cp_wuk0] + cp_ckv + [cp_wuv0]:
        c_.start()
    g_s[0:PAD, :] = jnp.zeros((PAD, M), f32)
    g_s[PAD + S:PAD + S + PAD, :] = jnp.zeros((PAD, M), f32)
    cv = jnp.broadcast_to(c_ref[...].astype(f32), (16, M))
    sil = (cv * jax.nn.sigmoid(cv)).astype(bf16)

    def relayout0(raw, dst):
        t = jnp.swapaxes(raw[...], 0, 1)
        for j in range(HG):
            dst[j] = t[j]

    cp_wuk0.wait()
    for c_ in cp_wmoda:
        c_.start()
    relayout0(wuk_raw0, wuk_t)
    for c_ in cp_ckv:
        c_.wait()
    cp_x[XC - 1].start()
    cp_wq0.start()
    for r in range(NB):
        lo, hi = r * BQ, (r + 1) * BQ
        k_s[lo:hi, :] = _mm(ckv_v[lo:hi, :], wuk_t[0]).astype(bf16)
    cp_wuv0.wait()
    wo_copy(0).start()
    cp_x[XC - 2].start()
    relayout0(wuv_raw0, wuv_t)
    for r in range(NB):
        lo, hi = r * BQ, (r + 1) * BQ
        v_s[lo:hi, :] = _mm(ckv_v[lo:hi, :], wuv_t[0]).astype(bf16)

    for c_ in cp_wmoda:
        c_.wait()
    for c_ in raw_copies(0) + cp_x[:XC - 2][::-1]:
        c_.start()
    mod_s[:, 0:2 * M] = _mm(sil, wmod_v[:, 0:2 * M])[0:8, :]

    def mod(i):
        return mod_s[0:1, i * M:(i + 1) * M]

    def norm_x(t):
        sa, ca = mod(0) * QSCALE, (1.0 + mod(1)) * QSCALE
        cp_x[t].wait()
        for r0 in range(t * XR, (t + 1) * XR, BQ):
            xr = x_v[r0:r0 + BQ, :].astype(f32)
            hr = (_ln(xr) * ca + sa).astype(bf16)
            for u in range(M // D):
                h_s[u, r0:r0 + BQ, :] = hr[:, u * D:(u + 1) * D]

    norm_x(XC - 1)
    cp_wq0.wait()
    relayout0(wq_raw0, wq_t)

    NRAW = NP - PPG

    def head(g, first):
        if not first:
            wo_copy(g).wait()

        def when(cond, fn):
            if first:
                if cond:
                    fn()
            else:
                pl.when(cond)(fn)

        def raw_wait():
            for c_ in raw_copies(g):
                c_.wait()

        def raw_start():
            for c_ in raw_copies(g + 1):
                c_.start()

        if not first:
            when(g < NRAW, raw_wait)
            when(g + 1 < NRAW, raw_start)
            when(g + 1 < NP, wo_copy(g + 1).start)
        for gi, c_ in enumerate((cp_wmodb, cp_w1, cp_w2, cp_w3, cp_w4)):
            when(g == gi + 1, c_.start)

        st = {}

        def pq(i):
            lo, hi = i * BQ, (i + 1) * BQ
            q_s[lo:hi, :] = _mm(_cat(h_s, lo, hi), wq_t[g]).astype(bf16)

        def pk(i):
            lo, hi = i * BQ, (i + 1) * BQ
            k_s[lo:hi, :] = _mm(ckv_v[lo:hi, :], wuk_t[g]).astype(bf16)

        def pv(i):
            lo, hi = i * BQ, (i + 1) * BQ
            v_s[lo:hi, :] = _mm(ckv_v[lo:hi, :], wuv_t[g]).astype(bf16)

        def po(i, gg):
            lo, hi = i * BQ, (i + 1) * BQ
            if first:
                acc_s[lo:hi, :] = _mm(ctx_s[lo:hi, :], wo_v[gg])
            else:
                acc_s[lo:hi, :] += _mm(ctx_s[lo:hi, :], wo_v[gg])

        def nkc(i):
            return i * BQ // KC

        def qk_chunk(i, c):
            lo = i * BQ
            d = st.setdefault(i, dict(s=[], mx=None))
            if c == 0:
                d['q'] = q_s[lo:lo + BQ, :]
            q = d['q']
            if c < nkc(i):
                sc = _mm_nt(q, k_s[c * KC:(c + 1) * KC, :])
                d['s'].append(sc)
                t = functools.reduce(jnp.maximum, [sc[:, u:u + D] for u in range(0, KC, D)])
                d['mx'] = t if d['mx'] is None else jnp.maximum(d['mx'], t)
            else:
                r = jax.lax.broadcasted_iota(jnp.int32, (D, D), 0)
                cc = jax.lax.broadcasted_iota(jnp.int32, (D, D), 1)
                tri = cc <= r
                mx = d['mx']
                tiles = []
                for t in range(BQ // D):
                    st_ = _mm_nt(q[t * D:], k_s[lo + t * D:lo + (t + 1) * D, :])
                    top = jnp.where(tri, st_[:D], NEG)
                    st_ = top if t == BQ // D - 1 else jnp.concatenate([top, st_[D:]], axis=0)
                    tiles.append(st_)
                    if mx is None:
                        mx = st_
                    elif t == 0:
                        mx = jnp.maximum(mx, st_)
                    else:
                        mx = jnp.concatenate([mx[:t * D], jnp.maximum(mx[t * D:], st_)], axis=0)
                d['s'].append(tiles)
                d['m'] = jnp.max(mx, axis=1, keepdims=True)

        def epv_chunk(i, c):
            lo = i * BQ
            d = st[i]
            m = d['m']
            if c < nkc(i):
                sc = d['s'][c]
                ps = [jnp.exp2(sc[:, u:u + D] - m) for u in range(0, KC, D)]
                pb = jnp.concatenate([p_.astype(bf16) for p_ in ps], axis=1)
                o = _mm(pb, v_s[c * KC:(c + 1) * KC, :])
                d['acc'] = o if c == 0 else d['acc'] + o
                t = functools.reduce(jnp.add, ps)
                d['l'] = t if c == 0 else d['l'] + t
            else:
                l = d['l'] if c > 0 else None
                acc = d['acc'] if c > 0 else None
                for t, st_ in enumerate(d['s'][c]):
                    p = jnp.exp2(st_ - m[t * D:])
                    o = _mm(p.astype(bf16), v_s[lo + t * D:lo + (t + 1) * D, :])
                    if l is None:
                        l, acc = p, o
                    elif t == 0:
                        l, acc = l + p, acc + o
                    else:
                        l = jnp.concatenate([l[:t * D], l[t * D:] + p], axis=0)
                        acc = jnp.concatenate([acc[:t * D], acc[t * D:] + o], axis=0)
                lsum = jnp.sum(l, axis=1, keepdims=True)
                ctx_s[lo:lo + BQ, :] = (acc / lsum).astype(bf16)

        def phase(qk_unit, epv_unit, fillers):
            nq = nkc(qk_unit) + 1 if qk_unit is not None else 0
            ne = nkc(epv_unit) + 1 if epv_unit is not None else 0
            n = max(nq, ne)
            nf = len(fillers)
            fpos = [((2 * t + 1) * n) // (2 * nf) for t in range(nf)]
            for c in range(n):
                if c < nq:
                    qk_chunk(qk_unit, c)
                for t in range(nf):
                    if fpos[t] == c:
                        fillers[t]()
                if c < ne:
                    epv_chunk(epv_unit, c)

        def relayout():
            slot = g % 2
            cidx = g % PPG
            for raw, dst, mc in ((wq_raw, wq_t, MQ), (wuk_raw, wuk_t, MK), (wuv_raw, wuv_t, MK)):
                t = jnp.swapaxes(raw[slot], 0, 1)
                r0 = pl.multiple_of(cidx * mc, 16)
                for j in range(HG):
                    pidx = ((g // PPG + 1) * PPG + j) % NP
                    dst[pidx, pl.ds(r0, mc), :] = t[j]

        P = functools.partial
        pq(ORDER[0])
        if not first:
            for c in range(LAG):
                pk(c)
            po(ORDER[-1], g - 1)
        pq(ORDER[1])
        for c in range(NB):
            if c + LAG < NB and not first:
                pk(c + LAG)
            qk_chunk(ORDER[0], c)
            if not first:
                pv(c)
        for n, i in enumerate(ORDER):
            if first:
                if n == 0:
                    wo_copy(0).wait()
                if n + 2 < NB and n % 2 == 0:
                    norm_x(XC - 2 - n // 2)
                if n == 2:
                    raw_start()
                    wo_copy(1).start()
                if n == TPOS:
                    raw_wait()
            f = []
            if n + 2 < NB:
                f += [P(pq, ORDER[n + 2])]
            if n >= 1:
                f += [P(po, ORDER[n - 1], g)]
            if n == TPOS:
                f += [relayout]
            phase(ORDER[n + 1] if n + 1 < NB else None, i, f)

    head(0, True)
    acc_s[ORDER[-1] * BQ:(ORDER[-1] + 1) * BQ, :] = jnp.zeros((BQ, M), f32)

    def body(g, carry):
        head(g, False)
        return carry

    jax.lax.fori_loop(1, NP, body, 0)

    for c_ in (cp_wmodb, cp_w1, cp_w2, cp_w3, cp_w4):
        c_.wait()
    lo_, hi_ = ORDER[-1] * BQ, (ORDER[-1] + 1) * BQ
    acc_s[lo_:hi_, :] += _mm(ctx_s[lo_:hi_, :], wo_v[NP - 1])
    mod_s[:, 2 * M:6 * M] = _mm(sil, wmod_v[:, 2 * M:6 * M])[0:8, :]
    ga, sb, cb, gb = mod(2), mod(3), mod(4), mod(5)
    NR = S // BM
    lane = jax.lax.broadcasted_iota(jnp.int32, (BM, 128), 1)
    cp_out = [cp(16 + r, out_v.at[r * BM:(r + 1) * BM, :], out_hbm.at[0, r * BM:(r + 1) * BM, :])
              for r in range(NR)]
    fchunks = [(lo, min(lo + FC, F)) for lo in range(0, F, FC)]
    sv = {}

    def stage1(r):
        lo, hi = r * BM, (r + 1) * BM
        x1 = x_v[lo:hi, :].astype(f32) + ga * acc_s[lo:hi, :]
        hb = _ln(x1) * (1.0 + cb) + sb
        acc_s[lo:hi, :] = x1
        hb_s[lo:hi, :] = hb
        u = _ln(hb).astype(bf16)
        g_s[PAD + lo:PAD + hi, :] = _gelu(_mm(u, w1_v[...]))

    def mix(r):
        lo, hi = r * BM, (r + 1) * BM

        def sh(d, t):
            return g_s[PAD + lo + d:PAD + hi + d, t * 128:(t + 1) * 128]

        t0 = sh(-1, 0)
        t1 = jnp.where(lane < 32, sh(-1, 1), sh(1, 1))
        t2 = jnp.where(lane < 64, sh(1, 2), sh(-2, 2))
        t3 = jnp.where(lane < 96, sh(-2, 3), sh(2, 3))
        t4 = sh(2, 4)
        gs = jnp.concatenate([t0, t1, t2, t3, t4], axis=1).astype(bf16)
        sv[r] = dict(xb=hb_s[lo:hi, :] + _mm(gs, w2_v[...]))

    def norm(r):
        sv[r]['u'] = _ln(sv[r]['xb']).astype(bf16)

    def up(r, c):
        lo, hi = fchunks[c]
        sv[r][('h', c)] = _mm_nt(sv[r]['u'], w3_v[lo:hi, :])

    def down(r, c):
        lo, hi = fchunks[c]
        o = _mm(_gelu(sv[r][('h', c)]).astype(bf16), w4_v[lo:hi, :])
        sv[r]['o'] = o if c == 0 else sv[r]['o'] + o

    def finish(r):
        lo, hi = r * BM, (r + 1) * BM
        out_v[lo:hi, :] = (acc_s[lo:hi, :] + gb * (sv[r]['xb'] + sv[r]['o'])).astype(bf16)
        cp_out[r].start()

    nc = len(fchunks)
    for r in range(3):
        stage1(r)
    for r in range(2):
        mix(r)
    for r in range(2):
        norm(r)
    up(0, 0)
    for r in range(NR):
        for c in range(nc):
            if c + 1 < nc:
                up(r, c + 1)
            elif r + 1 < NR:
                up(r + 1, 0)
            if c == 0 and 3 <= r + 2 < NR:
                stage1(r + 2)
            if c == 1 and 2 <= r + 1 < NR:
                mix(r + 1)
            if c == 2 and 2 <= r + 1 < NR:
                norm(r + 1)
            down(r, c)
        finish(r)
    for r in range(NR):
        cp_out[r].wait()


@jax.jit
def pallas_adaLN_cond__compressed_kv_cla__mixer_s_mlp__prompt_kernel(
    A_x: jax.Array,
    A_c_kv: jax.Array,
    A_w_q: jax.Array,
    A_w_uk: jax.Array,
    A_w_uv: jax.Array,
    A_w_o: jax.Array,
    B_x: jax.Array,
    B_w1: jax.Array,
    B_w2: jax.Array,
    B_w3: jax.Array,
    B_w4: jax.Array,
    c: jax.Array,
    w_mod: jax.Array,
):
    del B_x
    any_spec = pl.BlockSpec(memory_space=pltpu.HBM)
    V = pltpu.VMEM
    scratch = [
        V((S, M), bf16), V((S, DC), bf16),
        V((M, HG, D), bf16), V((DC, HG, D), bf16), V((DC, HG, D), bf16),
        V((2, M // PPG, HG, D), bf16), V((2, DC // PPG, HG, D), bf16), V((2, DC // PPG, HG, D), bf16),
        V((NP, D, M), bf16),
        V((M, M), bf16), V((M, M), bf16), V((F, M), bf16), V((F, M), bf16), V((M, 6 * M), bf16),
        V((NP, M, D), bf16), V((NP, DC, D), bf16), V((NP, DC, D), bf16),
        V((8, 6 * M), f32), V((M // D, S, D), bf16),
        V((S, D), bf16), V((S, D), bf16), V((S, D), bf16), V((S, D), bf16),
        V((S, M), f32), V((S, M), f32), V((S + 2 * PAD, M), f32), V((S, M), bf16),
        pltpu.SemaphoreType.DMA((16 + S // BM,)),
        pltpu.SemaphoreType.DMA((2, 4)),
    ]
    out = pl.pallas_call(
        _kernel,
        out_shape=jax.ShapeDtypeStruct((1, S, M), bf16),
        in_specs=[pl.BlockSpec(memory_space=pltpu.VMEM)] + [any_spec] * 11,
        out_specs=any_spec,
        scratch_shapes=scratch,
        compiler_params=pltpu.CompilerParams(
            vmem_limit_bytes=120 * 1024 * 1024,
            disable_bounds_checks=True,
        ),
    )(c, A_x.reshape(S, M), A_c_kv.reshape(S, DC), A_w_q, A_w_uk, A_w_uv, A_w_o.reshape(NP, D, M),
      B_w1, B_w2, B_w3.T, B_w4, w_mod)
    return out
```
